```python
import jax
import jax.numpy as jnp

def _softmax(x, axis=-1):
    return jax.nn.softmax(x, axis=axis)
def _gelu(x):
    return jax.nn.gelu(x, approximate=True)
def _silu(x):
    return jax.nn.silu(x)
def _sigmoid(x):
    return jax.nn.sigmoid(x)
def _layernorm(x, axis=-1, eps=1e-5):
    m = jnp.mean(x, axis=axis, keepdims=True)
    v = jnp.var(x, axis=axis, keepdims=True)
    return (x - m) / jnp.sqrt(v + eps)
def _scatter_add(tgt, idx, src, axis=0):
    return tgt.at[idx].add(src)
def _segment_sum(src, seg, n):
    return jax.ops.segment_sum(src, seg, n)
class _Rng:
    def __init__(self, key):
        self._k = key
    def _next(self):
        self._k, sub = jax.random.split(self._k)
        return sub
    def normal(self, shape):
        return jax.random.normal(self._next(), shape, dtype=jnp.bfloat16)
    def randint(self, lo, hi, shape):
        return jax.random.randint(self._next(), shape, lo, hi, dtype=jnp.int32)
    def uniform(self, shape, lo=0.0, hi=1.0):
        return jax.random.uniform(self._next(), shape, jnp.bfloat16, lo, hi)
    def permutation(self, n):
        return jax.random.permutation(self._next(), n)


kernel_name = 'gated_mix__ssm_conv_h3__sliding_local_dilated__prompt'

def setup_inputs():
    _rng = _Rng(jax.random.key(int.from_bytes(__import__("os").urandom(4), "little")))
    _w = (lambda a: (lambda t: t.astype(jnp.bfloat16) if jnp.issubdtype(t.dtype, jnp.floating) else t)(jnp.asarray(a)))
    def _A_setup():
        B, S, D = 1, 2048, 640
        ks = 4
        return {
            "q": _w((lambda *s: _rng.normal(s) * 0.05)(B, S, D)),
            "k": _w((lambda *s: _rng.normal(s) * 0.05)(B, S, D)),
            "v": _w((lambda *s: _rng.normal(s) * 0.05)(B, S, D)),
            "shift_k": _w((lambda *s: _rng.normal(s) * 0.05)(D, ks) * 0.5),
            "ssm_k": _w((lambda *s: _rng.normal(s) * 0.05)(D, S) * (1.0 / S ** 0.5)),
            "ssm_D": _w((lambda *s: _rng.normal(s) * 0.05)(D)),
        }
    _A_in = _A_setup()

    def _B_setup():
        B, S, D = 1, 2048, 640
        return {
            "x": _w((lambda *s: _rng.normal(s) * 0.05)(B, S, D)),
            "wqkv": _w((lambda *s: _rng.normal(s) * 0.05)(D, 3 * D)),
            "wo": _w((lambda *s: _rng.normal(s) * 0.05)(D, D)),
        }
    _B_in = _B_setup()

    return {
        "A_q": _A_in["q"],
        "A_k": _A_in["k"],
        "A_v": _A_in["v"],
        "A_shift_k": _A_in["shift_k"],
        "A_ssm_k": _A_in["ssm_k"],
        "A_ssm_D": _A_in["ssm_D"],
        "B_x": _B_in["x"],
        "B_wqkv": _B_in["wqkv"],
        "B_wo": _B_in["wo"],
        "gate_w": _w((lambda *s: _rng.normal(s) * 0.05)(640)),
    }

def reference(A_q, A_k, A_v, A_shift_k, A_ssm_k, A_ssm_D, B_x, B_wqkv, B_wo, gate_w):
    def _A_ref(q, k, v, shift_k, ssm_k, ssm_D):
        B, S, D = q.shape
        ks = shift_k.shape[-1]
        k_pad = jnp.pad(k, ((0, 0), (ks - 1, 0), (0, 0)))
        k_shift = jnp.zeros_like(k)
        for t in range(ks):
            k_shift = k_shift + k_pad[:, t:t + S, :] * shift_k[:, ks - 1 - t][None, None, :]
        kv = k_shift * v
        L = 2 * S
        kv_pad = jnp.pad(kv, ((0, 0), (0, S), (0, 0)))
        kf_pad = jnp.pad(ssm_k, ((0, 0), (0, S)))
        kv_f = (lambda x, axes=(-2,-1): jnp.fft.rfft2(x.astype(jnp.float32), axes=axes))(kv_pad[:, None, :, :], axes=(1, 2))
        kf_f = (lambda x, axes=(-2,-1): jnp.fft.rfft2(x.astype(jnp.float32), axes=axes))(kf_pad[:, None, :], axes=(1, 2))
        kf_f = (lambda x, *d: x.transpose(*d))(kf_f, 1, 2, 0)
        y_f = kv_f * kf_f[None, :, :, :]
        y = (lambda x, s, axes=(-2,-1): jnp.fft.irfft2(x, s=s, axes=axes).astype(jnp.bfloat16))(y_f, (1, L), axes=(1, 2))[:, 0, :S, :]
        y = y + kv * ssm_D[None, None, :]
        return q * y

    def _B_ref(x, wqkv, wo):
        B, S, D = x.shape
        H = 32; Dh = D // H
        W, dil = 8, 2
        qkv = (lambda x, *d: x.transpose(*d))((x @ wqkv).reshape(B, S, 3, H, Dh), 2, 0, 3, 1, 4)
        q, k, v = qkv[0], qkv[1], qkv[2]
        scale = Dh ** -0.5
        pos = jnp.arange(S)
        off = jnp.arange(W) * dil
        idx = pos[:, None] - off[None, :]
        mask = idx >= 0
        idx_c = jnp.where(mask, idx, 0).reshape(-1)
        kg = k[:, :, idx_c, :].reshape(B, H, S, W, Dh)
        vg = v[:, :, idx_c, :].reshape(B, H, S, W, Dh)
        logits = jnp.einsum("bhsd,bhswd->bhsw", q, kg) * scale
        logits = jnp.where(mask[None, None, :, :], logits, -1e9)
        attn = _softmax(logits, axis=-1)
        o = jnp.einsum("bhsw,bhswd->bhsd", attn, vg)
        return (lambda x, *d: x.transpose(*d))(o, 0, 2, 1, 3).reshape(B, S, D) @ wo

    x = A_q
    g = _sigmoid((x * gate_w).sum(-1, keepdims=True))
    a = _A_ref(x, A_k, A_v, A_shift_k, A_ssm_k, A_ssm_D)
    b = _B_ref(x, B_wqkv, B_wo)
    return g * a + (1 - g) * b
```

```python
import numpy as np

import jax
import jax.numpy as jnp
import jax.experimental.pallas as pl
import jax.experimental.pallas.tpu as pltpu

S, D = 2048, 640
H, DH = 32, 20
WIN, DIL = 8, 2
KS = 4
LANES = 128
NT = D // LANES
C = 128
NC = S // C
TB = 256
NB = S // TB
HALO = 16
AR = 16

F32 = jnp.float32
BF16 = jnp.bfloat16
NT_DIMS = (((1,), (1,)), ((), ()))


def _dft_matrices():
    f = np.concatenate([np.arange(0, C, 2), np.arange(1, C, 2)]).astype(np.float64)
    theta = 2.0 * np.pi * (f + 0.5) / (2 * C)
    ang = theta[:, None] * np.arange(C, dtype=np.float64)[None, :]
    fwd = np.concatenate([np.cos(ang), -np.sin(ang)], axis=0)
    inv = fwd.T / C
    return fwd.astype(BF16), inv.astype(BF16)


def _interleave(*lists):
    keyed = []
    for li, items in enumerate(lists):
        for i, item in enumerate(items):
            keyed.append(((i + 0.5) / len(items), li, i, item))
    keyed.sort(key=lambda t: t[:3])
    return [t[3] for t in keyed]


def _kernel(x_hbm, k_hbm, v_hbm, sk_ref, h_hbm, d_ref, wqkv_hbm, wo_hbm, gw_ref,
            f_ref, g_ref, out_hbm,
            x_v, k_v, v_v, h_v, wqkv_v, wo_v, out_v,
            wt_s, wp_s, wop_s, q_s, kk_s, vv_s, o_s, b_s,
            kf_s, xh_s, kh_s, yh_s, y_s, in_sem, out_sem):
    copies = {}

    def add_copy(name, src, dst):
        copies[name] = pltpu.make_async_copy(src, dst, in_sem.at[len(copies)])

    def add_x(s):
        rows = pl.ds(s * TB, TB)
        add_copy(("x", s), x_hbm.at[rows, :], x_v.at[rows, :])

    def add_w(p):
        cols = pl.ds(p * D, D)
        add_copy(("w", p), wqkv_hbm.at[:, cols], wqkv_v.at[p])

    def add_tile(c):
        cols = pl.ds(c * LANES, LANES)
        add_copy(("h", c), h_hbm.at[cols, :], h_v.at[c])
        add_copy(("k", c), k_hbm.at[:, cols], k_v.at[c])
        add_copy(("v", c), v_hbm.at[:, cols], v_v.at[c])

    add_w(0), add_x(0), add_w(1), add_w(2), add_x(1), add_tile(0)
    add_copy("wo", wo_hbm, wo_v)
    add_x(2), add_tile(1), add_x(3), add_tile(2), add_x(4), add_tile(3)
    add_x(5), add_tile(4), add_x(6), add_x(7)
    for cp in copies.values():
        cp.start()

    def out_copy(s):
        rows = pl.ds(s * TB, TB)
        return pltpu.make_async_copy(out_v.at[rows, :], out_hbm.at[rows, :], out_sem.at[s])

    def permute_rows(dst):
        for j in range(NT):
            for d in range(DH):
                rows = wt_s[j, pl.ds(d, H, stride=DH), :]
                dst[pl.ds(d * H, H), pl.ds(j * LANES, LANES)] = rows.astype(BF16)

    def prep_wqkv(p):
        for j in range(NT):
            for c in range(NT):
                blk = wqkv_v[p, pl.ds(j * LANES, LANES), pl.ds(c * LANES, LANES)]
                wt_s[j, pl.ds(c * LANES, LANES), :] = blk.T.astype(F32)
        permute_rows(wp_s.at[p])

    def prep_wo():
        for j in range(NT):
            wt_s[j] = wo_v[:, pl.ds(j * LANES, LANES)].astype(F32)
        permute_rows(wop_s)

    def proj_items(s):
        def item(p, c):
            def run():
                xb = x_v[pl.ds(s * TB, TB), :]
                w = wp_s[p, pl.ds(c * LANES, LANES), :]
                r = jax.lax.dot_general(xb, w, NT_DIMS, preferred_element_type=F32)
                if p == 0:
                    q_s[c, pl.ds(s * TB, TB), :] = r
                else:
                    dst = kk_s if p == 1 else vv_s
                    dst[c, pl.ds(HALO + s * TB, TB), :] = r
                    if s == 0:
                        dst[c, pl.ds(0, HALO), :] = jnp.broadcast_to(r[0:1, :], (HALO, LANES))
            return run
        return [item(p, c) for p in range(3) for c in range(NT)]

    def attn_items(s):
        scale = DH ** -0.5

        def item(t0):
            def run():
                q = [q_s[c, pl.ds(t0, AR), :] * scale for c in range(NT)]
                logits = []
                for w in range(WIN):
                    r0 = HALO + t0 - DIL * w
                    acc = q[0] * kk_s[0, pl.ds(r0, AR), :]
                    for c in range(1, NT):
                        acc = acc + q[c] * kk_s[c, pl.ds(r0, AR), :]
                    acc = acc + pltpu.roll(acc, 2 * H, 1)
                    acc = acc + pltpu.roll(acc, H, 1)
                    if t0 < DIL * w:
                        t = t0 + jax.lax.broadcasted_iota(jnp.int32, (AR, LANES), 0)
                        acc = jnp.where(t >= DIL * w, acc, -1e9)
                    logits.append(acc)
                m = logits[0]
                for w in range(1, WIN):
                    m = jnp.maximum(m, logits[w])
                p = [jnp.exp(l - m) for l in logits]
                den = p[0]
                for w in range(1, WIN):
                    den = den + p[w]
                inv = 1.0 / den
                for c in range(NT):
                    acc = p[0] * vv_s[c, pl.ds(HALO + t0, AR), :]
                    for w in range(1, WIN):
                        acc = acc + p[w] * vv_s[c, pl.ds(HALO + t0 - DIL * w, AR), :]
                    o_s[pl.ds(t0, AR), pl.ds(c * LANES, LANES)] = (acc * inv).astype(BF16)
            return run
        return [item(s * TB + i * AR) for i in range(TB // AR)]

    def wo_items(s):
        def item(c):
            def run():
                rows, cols = pl.ds(s * TB, TB), pl.ds(c * LANES, LANES)
                b_s[rows, cols] = jnp.dot(o_s[rows, :], wop_s[:, cols],
                                          preferred_element_type=F32)
            return run
        return [item(c) for c in range(NT)]

    def fwd_items(c):
        cols = pl.ds(c * LANES, LANES)
        slot = c % 2

        def h_item(m):
            def run():
                blk = h_v[c, :, pl.ds(m * C, C)]
                kh_s[slot, m] = jax.lax.dot_general(f_ref[...], blk, NT_DIMS,
                                                    preferred_element_type=F32)
            return run

        def kv_item(m):
            def run():
                if m == 0:
                    kf_s[pl.ds(0, 8), :] = jnp.zeros((8, LANES), F32)
                kf_s[pl.ds(8 + m * C, C), :] = k_v[c, pl.ds(m * C, C), :].astype(F32)
                taps = sk_ref[:, cols].astype(F32)
                acc = kf_s[pl.ds(8 + m * C, C), :] * taps[0:1, :]
                for j in range(1, KS):
                    acc = acc + kf_s[pl.ds(8 + m * C - j, C), :] * taps[j:j + 1, :]
                kv = acc * v_v[c, pl.ds(m * C, C), :].astype(F32)
                xh_s[slot, m] = jnp.dot(f_ref[...], kv.astype(BF16),
                                        preferred_element_type=F32)
            return run
        return [it(m) for m in range(NC) for it in (h_item, kv_item)]

    def mac_items(c):
        slot = c % 2

        def conv(a, b):
            out = []
            for i in range(NC):
                acc = a[i] * b[0]
                for j in range(1, i + 1):
                    acc = acc + a[i - j] * b[j]
                out.append(acc)
            return out

        def item(r):
            def run():
                re, im = pl.ds(8 * r, 8), pl.ds(C + 8 * r, 8)
                skip = jnp.broadcast_to(d_ref[:, pl.ds(c * LANES, LANES)].astype(F32), (8, LANES))
                kr = [kh_s[slot, m, re, :] for m in range(NC)]
                ki = [kh_s[slot, m, im, :] for m in range(NC)]
                if r < C // 16:
                    kc = [kr[0] + skip] + [kr[m] - ki[m - 1] for m in range(1, NC)]
                    kd = [ki[0]] + [ki[m] + kr[m - 1] for m in range(1, NC)]
                else:
                    kc = [kr[0] + skip] + [kr[m] + ki[m - 1] for m in range(1, NC)]
                    kd = [ki[0]] + [ki[m] - kr[m - 1] for m in range(1, NC)]
                t1 = conv(kc, [xh_s[slot, j, re, :] + xh_s[slot, j, im, :] for j in range(NC)])
                t2 = conv([kd[m] - kc[m] for m in range(NC)],
                          [xh_s[slot, j, re, :] for j in range(NC)])
                for i in range(NC):
                    yh_s[slot, i, im, :] = t1[i] + t2[i]
                t3 = conv([kd[m] + kc[m] for m in range(NC)],
                          [xh_s[slot, j, im, :] for j in range(NC)])
                for i in range(NC):
                    yh_s[slot, i, re, :] = t1[i] - t3[i]
            return run
        return [item(r) for r in range(C // 8)]

    def inv_items(c):
        slot = c % 2

        def item(i):
            def run():
                y_s[pl.ds(i * C, C), pl.ds(c * LANES, LANES)] = jnp.dot(
                    g_ref[...], yh_s[slot, i].astype(BF16), preferred_element_type=F32)
            return run
        return [item(i) for i in range(NC)]

    def mix_items(s):
        def item(t0):
            def run():
                rows = pl.ds(t0, AR)
                x = x_v[rows, :].astype(F32)
                z = jnp.sum(x * gw_ref[...].astype(F32), axis=-1, keepdims=True)
                gate = 1.0 / (1.0 + jnp.exp(-z))
                b = b_s[rows, :]
                out_v[rows, :] = (gate * (x * y_s[rows, :] - b) + b).astype(out_v.dtype)
            return run
        return [item(s * TB + i * AR) for i in range(TB // AR)]

    mix_at = {NB: list(range(NB - 2)), NB + 1: [NB - 2, NB - 1]}
    for step in range(NB + 2):
        lists = []
        if step == 0:
            items = proj_items(0)
            for p in range(3):
                copies["w", p].wait()
                prep_wqkv(p)
                if p == 0:
                    copies["x", 0].wait()
                for run in items[p * NT:(p + 1) * NT]:
                    run()
            continue
        if step < NB:
            copies["x", step].wait()
            lists.append(proj_items(step))
        if step == 2:
            copies["wo"].wait()
            prep_wo()
        if 0 <= step - 2 < NB:
            lists.append(wo_items(step - 2))
        if 0 <= step - 1 < NT:
            for name in "hkv":
                copies[name, step - 1].wait()
            lists.append(fwd_items(step - 1))
        if 0 <= step - 3 < NT:
            lists.append(inv_items(step - 3))
        if 0 <= step - 1 < NB:
            lists.append(attn_items(step - 1))
        if 0 <= step - 2 < NT:
            lists.append(mac_items(step - 2))
        if step == NB + 1:
            for run in _interleave(*lists):
                run()
            lists = []
        for s in mix_at.get(step, []):
            lists.append(mix_items(s))
        for run in _interleave(*lists):
            run()
        for s in mix_at.get(step, []):
            out_copy(s).start()
    for s in range(NB):
        out_copy(s).wait()


@jax.jit
def pallas_gated_mix__ssm_conv_h3__sliding_local_dilated__prompt_kernel(
    A_q: jax.Array,
    A_k: jax.Array,
    A_v: jax.Array,
    A_shift_k: jax.Array,
    A_ssm_k: jax.Array,
    A_ssm_D: jax.Array,
    B_x: jax.Array,
    B_wqkv: jax.Array,
    B_wo: jax.Array,
    gate_w: jax.Array,
):
    del B_x
    fwd, inv = _dft_matrices()
    hbm = pl.BlockSpec(memory_space=pl.ANY)
    vmem = pl.BlockSpec(memory_space=pltpu.VMEM)
    out = pl.pallas_call(
        _kernel,
        out_shape=jax.ShapeDtypeStruct((S, D), A_q.dtype),
        in_specs=[hbm, hbm, hbm, vmem, hbm, vmem, hbm, hbm, vmem, vmem, vmem],
        out_specs=hbm,
        scratch_shapes=[
            pltpu.VMEM((S, D), BF16),
            pltpu.VMEM((NT, S, LANES), BF16),
            pltpu.VMEM((NT, S, LANES), BF16),
            pltpu.VMEM((NT, LANES, S), BF16),
            pltpu.VMEM((3, D, D), BF16),
            pltpu.VMEM((D, D), BF16),
            pltpu.VMEM((S, D), A_q.dtype),
            pltpu.VMEM((NT, D, LANES), F32),
            pltpu.VMEM((3, D, D), BF16),
            pltpu.VMEM((D, D), BF16),
            pltpu.VMEM((NT, S, LANES), F32),
            pltpu.VMEM((NT, HALO + S, LANES), F32),
            pltpu.VMEM((NT, HALO + S, LANES), F32),
            pltpu.VMEM((S, D), BF16),
            pltpu.VMEM((S, D), F32),
            pltpu.VMEM((8 + S, LANES), F32),
            pltpu.VMEM((2, NC, 2 * C, LANES), F32),
            pltpu.VMEM((2, NC, 2 * C, LANES), F32),
            pltpu.VMEM((2, NC, 2 * C, LANES), F32),
            pltpu.VMEM((S, D), F32),
            pltpu.SemaphoreType.DMA((NB + 4 + 3 * NT,)),
            pltpu.SemaphoreType.DMA((NB,)),
        ],
        compiler_params=pltpu.CompilerParams(vmem_limit_bytes=110 * 1024 * 1024),
    )(
        A_q.reshape(S, D), A_k.reshape(S, D), A_v.reshape(S, D),
        A_shift_k.T, A_ssm_k, A_ssm_D.reshape(1, D), B_wqkv, B_wo,
        gate_w.reshape(1, D), fwd, inv,
    )
    return out.reshape(A_q.shape)
```

```python
import numpy as np

import jax
import jax.numpy as jnp
import jax.experimental.pallas as pl
import jax.experimental.pallas.tpu as pltpu

S, D = 2048, 640
H, DH = 32, 20
WIN, DIL = 8, 2
KS = 4
LANES = 128
NT = D // LANES
C = 128
NC = S // C
R = 4
NJ = S // (R * C)
TB = 256
NB = S // TB
HALO = 16
MR = 32
AR = 16

LOG2E = float(np.log2(np.e))
F32 = jnp.float32
BF16 = jnp.bfloat16
U32 = jnp.uint32
NT_DIMS = (((1,), (1,)), ((), ()))


def _as_words(mat):
    bits = mat.astype(np.float32).astype(BF16).view(np.uint16).astype(np.uint32)
    return bits[0::2] | (bits[1::2] << 16)


def _dft_matrices():
    f = np.concatenate([np.arange(0, C, 2), np.arange(1, C, 2)]).astype(np.float64)
    theta = 2.0 * np.pi * (f + 0.5) / (2 * R * C)
    fwd, inv = [], []
    for j in range(R):
        ang = theta[:, None] * (R * np.arange(C, dtype=np.float64) + j)[None, :]
        mat = np.stack([np.cos(ang).reshape(C // 8, 8, C), -np.sin(ang).reshape(C // 8, 8, C)],
                       axis=1).reshape(2 * C, C)
        fwd.append(mat)
        inv += [mat[:C].T / (R * C), mat[C:].T / (R * C)]
    return _as_words(np.concatenate(fwd, axis=0)), _as_words(np.concatenate(inv, axis=0))


def _lo(words):
    return pltpu.bitcast(words << 16, F32)


def _hi(words):
    return pltpu.bitcast(words & np.uint32(0xFFFF0000), F32)


def _cadd(a, b):
    return a[0] + b[0], a[1] + b[1]


def _csub(a, b):
    return a[0] - b[0], a[1] - b[1]


def _cadd_i(a, b):
    return a[0] - b[1], a[1] + b[0]


def _csub_i(a, b):
    return a[0] + b[1], a[1] - b[0]


def _pairs(mat):
    return [(mat[r:r + 8], mat[r + 8:r + 16]) for r in range(0, mat.shape[0], 16)]


def _dft4(mats, sign):
    plus, minus = (_cadd_i, _csub_i) if sign > 0 else (_csub_i, _cadd_i)
    out = [[] for _ in mats]
    for e in zip(*map(_pairs, mats)):
        a, b = _cadd(e[0], e[2]), _csub(e[0], e[2])
        c, d = _cadd(e[1], e[3]), _csub(e[1], e[3])
        for rows, val in zip(out, (_cadd(a, c), plus(b, d), _csub(a, c), minus(b, d))):
            rows.extend(val)
    return [jnp.concatenate(rows, axis=0) for rows in out]


def _cmul(a, b):
    return a[0] * b[0] - a[1] * b[1], a[0] * b[1] + a[1] * b[0]


def _ld16(ref, r0, n):
    return pltpu.bitcast(ref[pl.ds(r0 // 2, n // 2), :], BF16)


def _st16(ref, r0, value):
    ref[pl.ds(r0 // 2, value.shape[0] // 2), :] = pltpu.bitcast(value.astype(BF16), U32)


def _interleave(*lists):
    keyed = []
    for li, items in enumerate(lists):
        for i, item in enumerate(items):
            keyed.append(((i + 0.5) / len(items), li, i, item))
    keyed.sort(key=lambda t: t[:3])
    return [t[3] for t in keyed]


def _aligned(index, multiple):
    return index if isinstance(index, int) else pl.multiple_of(index, multiple)


def _kernel(x_hbm, k_hbm, v_hbm, sk_ref, h_hbm, d_ref, wqkv_hbm, wo_hbm, gw_ref,
            f_ref, g_ref, out_hbm,
            x_v, k_v, v_v, h_v, w_v, out_v, wt_s, wp_s, qkv_s, stage_s, o_s, b_s, ht_s,
            xh0_s, xh1_s, kh0_s, kh1_s, yh0_s, yh1_s, y_s, gate_s, vec_s,
            x_sem, w_sem, t_sem, stage_sem, out_sem):
    xh_s, kh_s, yh_s = (xh0_s, xh1_s), (kh0_s, kh1_s), (yh0_s, yh1_s)

    def lane_tile(c):
        return pl.ds(_aligned(c * LANES, LANES), LANES)

    def x_copies(s):
        rows = pl.ds(_aligned(s * TB, TB), TB)
        return [pltpu.make_async_copy(x_hbm.at[rows, lane_tile(c)],
                                      x_v.bitcast(BF16).at[c, rows, :], x_sem.at[s, c])
                for c in range(NT)]

    def w_copies(p):
        src = wo_hbm if p == 3 else wqkv_hbm
        return [pltpu.make_async_copy(src.at[:, lane_tile(p % 3 * NT + c)],
                                      w_v.bitcast(BF16).at[p, c], w_sem.at[p, c])
                for c in range(NT)]

    def tile_copies(c):
        cps = [pltpu.make_async_copy(h_hbm.at[lane_tile(c), pl.ds(jj * R * C, R * C)],
                                     h_v.bitcast(BF16).at[c, jj], t_sem.at[c, jj])
               for jj in range(NJ)]
        cps.append(pltpu.make_async_copy(k_hbm.at[:, lane_tile(c)],
                                         k_v.bitcast(BF16).at[c, pl.ds(16, S), :], t_sem.at[c, NJ]))
        cps.append(pltpu.make_async_copy(v_hbm.at[:, lane_tile(c)],
                                         v_v.bitcast(BF16).at[c], t_sem.at[c, NJ + 1]))
        return cps

    def out_copies(s):
        rows = pl.ds(_aligned(s * TB, TB), TB)
        return [pltpu.make_async_copy(out_v.bitcast(BF16).at[c, rows, :],
                                      out_hbm.at[rows, lane_tile(c)], out_sem.at[s, c])
                for c in range(NT)]

    def start(copies):
        for cp in copies:
            cp.start()

    def wait(copies):
        for cp in copies:
            cp.wait()

    def head_minor(j, d):
        return wt_s[j, pl.ds(d, H, stride=DH), :]

    def prep_wqkv(p):
        for j in range(NT):
            for c in range(NT):
                blk = _ld16(w_v.at[p, c], j * LANES, LANES)
                wt_s[j, pl.ds(c * LANES, LANES), :] = blk.T.astype(F32)
        for j in range(NT):
            for d in range(DH):
                _st16(wp_s.at[p, j], d * H, head_minor(j, d))

    def prep_wo():
        per = LANES // H
        for c in range(NT):
            wt_s[c] = _ld16(w_v.at[3, c], 0, D).astype(F32)
        for c in range(NT):
            for j in range(NT):
                blk = jnp.concatenate([head_minor(c, j * per + d) for d in range(per)], axis=0)
                _st16(wp_s.at[3, j], c * LANES, blk.astype(BF16).T)

    def dense_items(p, s, lhs_ref, dst):
        src = lhs_ref.at[:, pl.ds(_aligned(s * (TB // 2), TB // 2), TB // 2), :]
        last = NT - 1

        def head(c):
            def run():
                lhs = jnp.concatenate([_ld16(src.at[j], 0, TB) for j in range(last)], axis=1)
                w = jnp.concatenate([_ld16(wp_s.at[p, j], c * LANES, LANES)
                                     for j in range(last)], axis=1)
                dst[c] = jax.lax.dot_general(lhs, w, NT_DIMS, preferred_element_type=F32)
            return run

        def tail(c, r0, n):
            dst[c, pl.ds(r0, n), :] += jax.lax.dot_general(
                _ld16(src.at[last], r0, n), _ld16(wp_s.at[p, last], c * LANES, LANES),
                NT_DIMS, preferred_element_type=F32)

        def tails():
            for c in range(last):
                tail(c, 0, TB)

        def last_tail():
            for r0 in range(0, TB, TB // 4):
                tail(last, r0, TB // 4)

        return [head(c) for c in range(last)] + [tails, head(last), last_tail]

    def qkv_block(p, s):
        return qkv_s.at[p, :, pl.ds(_aligned(HALO + s * TB, 8), TB), :]

    def attn_items(t0, rows, first=False):
        scale = DH ** -0.5 * LOG2E
        win = qkv_s.at[:, :, pl.ds(_aligned(t0, 8), HALO + rows), :]
        dst = o_s.at[:, pl.ds(_aligned(t0 // 2, 8), rows // 2), :]

        def item(r0):
            def run():
                q = [win[0, c, pl.ds(HALO + r0, AR), :] * scale for c in range(NT)]
                part = []
                for w in range(WIN):
                    taps = pl.ds(HALO + r0 - DIL * w, AR)
                    acc = q[0] * win[1, 0, taps, :]
                    for c in range(1, NT):
                        acc = acc + q[c] * win[1, c, taps, :]
                    part.append(acc)
                lane = jax.lax.broadcasted_iota(jnp.int32, (AR, LANES), 1)
                even = (lane & H) == 0
                logits = []
                for w in range(0, WIN, 2):
                    acc = (jnp.where(even, part[w], part[w + 1])
                           + pltpu.roll(jnp.where(even, part[w + 1], part[w]), H, 1))
                    acc = acc + pltpu.roll(acc, 2 * H, 1)
                    if first and r0 < DIL * (w + 1):
                        t = t0 + r0 + jax.lax.broadcasted_iota(jnp.int32, (AR, LANES), 0)
                        reach = jnp.where(even, DIL * w, DIL * (w + 1))
                        acc = jnp.where(t >= reach, acc, -1e9 * LOG2E)
                    logits.append(acc)
                m = logits[0]
                for l in logits[1:]:
                    m = jnp.maximum(m, l)
                m = jnp.maximum(m, pltpu.roll(m, H, 1))
                p = []
                for l in logits:
                    e = jnp.exp2(l - m)
                    other = pltpu.roll(e, H, 1)
                    p += [jnp.where(even, e, other), jnp.where(even, other, e)]
                den = p[0]
                for w in range(1, WIN):
                    den = den + p[w]
                inv = pltpu.reciprocal(den, full_range=False)
                for c in range(NT):
                    acc = p[0] * win[2, c, pl.ds(HALO + r0, AR), :]
                    for w in range(1, WIN):
                        acc = acc + p[w] * win[2, c, pl.ds(HALO + r0 - DIL * w, AR), :]
                    _st16(dst.at[c], r0, acc * inv)
            return run
        return [item(r0) for r0 in range(0, rows, AR)]

    def fwd_items(c, slot, jj):
        half = R * C // 2
        base = _aligned(jj * half, half)

        def dft(dst, tiles):
            parts = [jnp.dot(_ld16(f_ref, j * 2 * C, 2 * C), tile.astype(BF16),
                             preferred_element_type=F32) for j, tile in enumerate(tiles)]
            for k, spec in enumerate(_dft4(parts, -1)):
                dst[jj, k] = spec

        def h_item():
            for i in range(R):
                blk = pltpu.bitcast(h_v[c, jj, :, pl.ds(i * C, C)], BF16)
                ht_s[pl.ds(i * C // 2, C // 2), :] = pltpu.bitcast(blk.T, U32)
            words = [ht_s[pl.ds(j2, C, stride=2), :] for j2 in range(R // 2)]
            dft(kh_s[slot], [half_of(w) for w in words for half_of in (_lo, _hi)])

        def kv_item():
            taps = vec_s[c]
            kc = k_v.at[c, pl.ds(base, 8 + half), :]
            vc = v_v.at[c, pl.ds(base, half), :]
            kw = [kc[pl.ds(8 + o, C, stride=2), :] for o in (-2, -1, 0, 1)]
            ks = [_hi(kw[0]), _lo(kw[1]), _hi(kw[1]), _lo(kw[2]), _hi(kw[2]),
                  _lo(kw[3]), _hi(kw[3])]
            tiles = []
            for j in range(R):
                vw = vc[pl.ds(j // 2, C, stride=2), :]
                acc = ks[3 + j] * taps[0:1, :]
                for t in range(1, KS):
                    acc = acc + ks[3 + j - t] * taps[t:t + 1, :]
                tiles.append(acc * (_hi(vw) if j % 2 else _lo(vw)))
            dft(xh_s[slot], tiles)

        return [h_item, kv_item]

    def mac_items(c, slot, u):
        xh, kh, yh = xh_s[slot], kh_s[slot], yh_s[slot]

        def item(i, k):
            def run():
                r0 = _aligned(16 * (NJ * i + u), 16)
                re, im = pl.ds(r0, 8), pl.ds(r0 + 8, 8)
                x = [(xh[jj, k, re, :], xh[jj, k, im, :]) for jj in range(NJ)]
                h = [(kh[jj, k, re, :], kh[jj, k, im, :]) for jj in range(NJ)]
                fold = _cadd_i if i < 2 else _csub_i
                h = ([(h[0][0] + vec_s[c, KS:KS + 1, :], h[0][1])]
                     + [fold(h[m], h[m - 1]) for m in range(1, NJ)])
                for jj in range(NJ):
                    acc = _cmul(h[jj], x[0])
                    for j in range(1, jj + 1):
                        acc = _cadd(acc, _cmul(h[jj - j], x[j]))
                    yh[jj, k, re, :] = acc[0]
                    yh[jj, k, im, :] = acc[1]
            return run
        return [item(i, k) for i in range(C // 8 // NJ) for k in range(R)]

    def inv_items(c, slot, jj):
        def run():
            spec = _dft4([yh_s[slot][jj, k] for k in range(R)], +1)
            dst = y_s.at[c, pl.ds(_aligned(jj * R * C, R * C), R * C), :]
            for j in range(R):
                g = jnp.concatenate([_ld16(g_ref, 2 * j * C, C),
                                     _ld16(g_ref, (2 * j + 1) * C, C)], axis=1)
                dst[pl.ds(j, C, stride=R), :] = jnp.dot(g, spec[j].astype(BF16),
                                                        preferred_element_type=F32)
        return [run]

    def gate_items(t0, rows):
        src = x_v.at[:, pl.ds(_aligned(t0 // 2, 8), rows // 2), :]
        dst = gate_s.at[pl.ds(_aligned(t0, 8), rows), :]

        def item(r0):
            def run():
                z = _ld16(src.at[0], r0, MR).astype(F32) * vec_s[0, KS + 1:KS + 2, :]
                for c in range(1, NT):
                    z = z + _ld16(src.at[c], r0, MR).astype(F32) * vec_s[c, KS + 1:KS + 2, :]
                z = jnp.sum(z, axis=-1, keepdims=True)
                dst[pl.ds(r0, MR), :] = jnp.broadcast_to(1.0 / (1.0 + jnp.exp(-z)), (MR, LANES))
            return run
        return [item(r0) for r0 in range(0, rows, MR)]

    def mix_items(s):
        words = pl.ds(_aligned(s * (TB // 2), TB // 2), TB // 2)
        rows = pl.ds(_aligned(s * TB, TB), TB)
        x, out = x_v.at[:, words, :], out_v.at[:, words, :]
        att, y, gates = b_s.at[:, rows, :], y_s.at[:, rows, :], gate_s.at[rows, :]

        def item(r0):
            def run():
                gate = gates[pl.ds(r0, MR), :]
                for c in range(NT):
                    b = att[c, pl.ds(r0, MR), :]
                    a = _ld16(x.at[c], r0, MR).astype(F32) * y[c, pl.ds(r0, MR), :]
                    _st16(out.at[c], r0, gate * (a - b) + b)
            return run
        return [item(r0) for r0 in range(0, TB, MR)]

    def emit(*lists):
        for run in _interleave(*lists):
            run()

    start(w_copies(0) + x_copies(0) + w_copies(1))
    small = jnp.concatenate([sk_ref[...].astype(F32), d_ref[...].astype(F32).reshape(1, D),
                             gw_ref[...].astype(F32).reshape(1, D), jnp.zeros((2, D), F32)], axis=0)
    for c in range(NT):
        vec_s[c] = small[:, c * LANES:(c + 1) * LANES]
        k_v[c, pl.ds(0, 8), :] = jnp.zeros((8, LANES), U32)
    wait(w_copies(0))
    start(w_copies(2) + x_copies(1))
    prep_wqkv(0)
    wait(x_copies(0) + w_copies(1))
    start(tile_copies(0))
    emit(dense_items(0, 0, x_v, qkv_block(0, 0)), [lambda: prep_wqkv(1)])
    wait(w_copies(2))
    start(w_copies(3) + x_copies(2))
    emit(dense_items(1, 0, x_v, qkv_block(1, 0)), [lambda: prep_wqkv(2)])
    wait(x_copies(1))
    emit(dense_items(2, 0, x_v, qkv_block(2, 0)))
    wait(w_copies(3))
    start(x_copies(3))
    emit(dense_items(0, 1, x_v, qkv_block(0, 1)), [prep_wo])
    for p in (1, 2):
        for c in range(NT):
            qkv_s[p, c, pl.ds(0, HALO), :] = jnp.broadcast_to(
                qkv_s[p, c, pl.ds(HALO, 1), :], (HALO, LANES))

    quarter = TB // NJ
    done = 4

    def stage_copy(i):
        return pltpu.make_async_copy(stage_s.at[i % 2], qkv_block((i + done) % 3, (i + done) // 3),
                                     stage_sem.at[i % 2])

    def tick(c, u, slot, mac, inv, first=False):
        i = c * NJ + u
        p, s = (i + done) % 3, (i + done) // 3

        @pl.when(i >= 2)
        def _():
            stage_copy(i - 2).wait()

        @pl.when(p == 0)
        def _():
            wait(x_copies(s))

            @pl.when(s + 2 < NB)
            def _():
                start(x_copies(s + 2))

        @pl.when(u == 0)
        def _():
            wait(tile_copies(c))

            @pl.when(c + 1 < NT)
            def _():
                start(tile_copies(c + 1))

        lists = [dense_items(p, s, x_v, stage_s.at[i % 2]), fwd_items(c, slot, u)]
        if inv:
            lists.append(inv_items(c - 2, slot, u))
        lists.append(attn_items(i * quarter, quarter, first))
        if mac:
            lists.append(mac_items(c - 1, 1 - slot, u))
        emit(*lists)
        stage_copy(i).start()

    def ticks(c, slot, **stages):
        pl.loop(0, NJ)(lambda u: tick(c, u, slot, **stages))

    ticks(0, 0, mac=False, inv=False, first=True)
    ticks(1, 1, mac=True, inv=False)

    @pl.loop(2, NT)
    def _(c):
        for slot in range(2):
            pl.when(c % 2 == slot)(lambda: ticks(c, slot, mac=True, inv=True))

    for i in (NT * NJ - 2, NT * NJ - 1):
        stage_copy(i).wait()

    def out_items(s):
        return dense_items(3, s, o_s, b_s.at[:, pl.ds(_aligned(s * TB, TB), TB), :])

    @pl.loop(0, NJ)
    def _(u):
        emit(out_items(u), inv_items(NT - 2, NT % 2, u),
             attn_items(NT * TB + u * 2 * quarter, 2 * quarter),
             mac_items(NT - 1, (NT - 1) % 2, u))

    def mix(u):
        return mix_items(2 * u) + mix_items(2 * u + 1)

    done_rows = (NB - 1) * TB
    for u, rows in enumerate((96, 80, 80, 0)):
        emit(out_items(NJ + u), inv_items(NT - 1, (NT - 1) % 2, u),
             attn_items(done_rows, rows) if rows else [], gate_items(u * (S // NJ), S // NJ),
             mix(u - 1) if u else [])
        done_rows += rows
        if u:
            start(out_copies(2 * u - 2) + out_copies(2 * u - 1))
    for s in (NB - 2, NB - 1):
        emit(mix_items(s))
        start(out_copies(s))
    for s in range(NB):
        wait(out_copies(s))


@jax.jit
def pallas_gated_mix__ssm_conv_h3__sliding_local_dilated__prompt_kernel(
    A_q: jax.Array,
    A_k: jax.Array,
    A_v: jax.Array,
    A_shift_k: jax.Array,
    A_ssm_k: jax.Array,
    A_ssm_D: jax.Array,
    B_x: jax.Array,
    B_wqkv: jax.Array,
    B_wo: jax.Array,
    gate_w: jax.Array,
):
    del B_x
    fwd, inv = _dft_matrices()
    hbm = pl.BlockSpec(memory_space=pl.ANY)
    vmem = pl.BlockSpec(memory_space=pltpu.VMEM)
    out = pl.pallas_call(
        _kernel,
        out_shape=jax.ShapeDtypeStruct((S, D), A_q.dtype),
        in_specs=[hbm, hbm, hbm, vmem, hbm, vmem, hbm, hbm, vmem, vmem, vmem],
        out_specs=hbm,
        scratch_shapes=[
            pltpu.VMEM((NT, S // 2, LANES), U32),
            pltpu.VMEM((NT, 8 + S // 2, LANES), U32),
            pltpu.VMEM((NT, S // 2, LANES), U32),
            pltpu.VMEM((NT, NJ, LANES // 2, R * C), U32),
            pltpu.VMEM((4, NT, D // 2, LANES), U32),
            pltpu.VMEM((NT, S // 2, LANES), U32),
            pltpu.VMEM((NT, D, LANES), F32),
            pltpu.VMEM((4, NT, D // 2, LANES), U32),
            pltpu.VMEM((3, NT, HALO + S, LANES), F32),
            pltpu.VMEM((2, NT, TB, LANES), F32),
            pltpu.VMEM((NT, S // 2, LANES), U32),
            pltpu.VMEM((NT, S, LANES), F32),
            pltpu.VMEM((R * C // 2, LANES), U32),
            *[pltpu.VMEM((NJ, R, 2 * C, LANES), F32)] * 6,
            pltpu.VMEM((NT, S, LANES), F32),
            pltpu.VMEM((S, LANES), F32),
            pltpu.VMEM((NT, 8, LANES), F32),
            pltpu.SemaphoreType.DMA((NB, NT)),
            pltpu.SemaphoreType.DMA((4, NT)),
            pltpu.SemaphoreType.DMA((NT, NJ + 2)),
            pltpu.SemaphoreType.DMA((2,)),
            pltpu.SemaphoreType.DMA((NB, NT)),
        ],
        compiler_params=pltpu.CompilerParams(vmem_limit_bytes=110 * 1024 * 1024),
    )(
        A_q.reshape(S, D), A_k.reshape(S, D), A_v.reshape(S, D),
        A_shift_k.T, A_ssm_k, A_ssm_D, B_wqkv, B_wo,
        gate_w, fwd, inv,
    )
    return out.reshape(A_q.shape)
```

```python
import numpy as np

import jax
import jax.numpy as jnp
import jax.experimental.pallas as pl
import jax.experimental.pallas.tpu as pltpu

S, D = 2048, 640
H, DH = 32, 20
WIN, DIL = 8, 2
KS = 4
LANES = 128
NT = D // LANES
C = 128
NC = S // C
R = 4
NJ = S // (R * C)
TB = 256
NB = S // TB
HALO = 16
O_SPLIT = 6
STAGES = 3
MR = 32
AR = 16

LOG2E = float(np.log2(np.e))
F32 = jnp.float32
BF16 = jnp.bfloat16
U32 = jnp.uint32
NT_DIMS = (((1,), (1,)), ((), ()))


def _as_words(mat):
    bits = mat.astype(np.float32).astype(BF16).view(np.uint16).astype(np.uint32)
    return bits[0::2] | (bits[1::2] << 16)


def _dft_matrices():
    f = np.concatenate([np.arange(0, C, 2), np.arange(1, C, 2)]).astype(np.float64)
    theta = 2.0 * np.pi * (f + 0.5) / (2 * R * C)
    fwd, inv = [], []
    for j in range(R):
        ang = theta[:, None] * (R * np.arange(C, dtype=np.float64) + j)[None, :]
        mat = np.stack([np.cos(ang).reshape(C // 8, 8, C), -np.sin(ang).reshape(C // 8, 8, C)],
                       axis=1).reshape(2 * C, C)
        fwd.append(mat)
        inv += [mat[:C].T / (R * C), mat[C:].T / (R * C)]
    return _as_words(np.concatenate(fwd, axis=0)), _as_words(np.concatenate(inv, axis=0))


def _lo(words):
    return pltpu.bitcast(words << 16, F32)


def _hi(words):
    return pltpu.bitcast(words & np.uint32(0xFFFF0000), F32)


def _cadd(a, b):
    return a[0] + b[0], a[1] + b[1]


def _csub(a, b):
    return a[0] - b[0], a[1] - b[1]


def _cadd_i(a, b):
    return a[0] - b[1], a[1] + b[0]


def _csub_i(a, b):
    return a[0] + b[1], a[1] - b[0]


def _pairs(mat):
    return [(mat[r:r + 8], mat[r + 8:r + 16]) for r in range(0, mat.shape[0], 16)]


def _dft4(mats, sign):
    plus, minus = (_cadd_i, _csub_i) if sign > 0 else (_csub_i, _cadd_i)
    out = [[] for _ in mats]
    for e in zip(*map(_pairs, mats)):
        a, b = _cadd(e[0], e[2]), _csub(e[0], e[2])
        c, d = _cadd(e[1], e[3]), _csub(e[1], e[3])
        for rows, val in zip(out, (_cadd(a, c), plus(b, d), _csub(a, c), minus(b, d))):
            rows.extend(val)
    return [jnp.concatenate(rows, axis=0) for rows in out]


def _cmul(a, b):
    return a[0] * b[0] - a[1] * b[1], a[0] * b[1] + a[1] * b[0]


def _ld16(ref, r0, n):
    return pltpu.bitcast(ref[pl.ds(r0 // 2, n // 2), :], BF16)


def _st16(ref, r0, value):
    ref[pl.ds(r0 // 2, value.shape[0] // 2), :] = pltpu.bitcast(value.astype(BF16), U32)


def _interleave(*lists):
    keyed = []
    for li, items in enumerate(lists):
        for i, item in enumerate(items):
            keyed.append(((i + 0.5) / len(items), li, i, item))
    keyed.sort(key=lambda t: t[:3])
    return [t[3] for t in keyed]


def _aligned(index, multiple):
    return index if isinstance(index, int) else pl.multiple_of(index, multiple)


def _kernel(x_hbm, k_hbm, v_hbm, sk_ref, h_hbm, d_ref, wqkv_hbm, wo_hbm, gw_ref,
            f_ref, g_ref, out_hbm,
            x_v, k_v, v_v, h_v, w_v, out_v, wt_s, wp_s, qkv_s, stage_s, o0_s, o1_s, b_s, ht_s,
            xh0_s, xh1_s, kh0_s, kh1_s, yh0_s, yh1_s, y_s, gate_s, vec_s,
            x_sem, w_sem, t_sem, stage_sem, out_sem):
    xh_s, kh_s, yh_s = (xh0_s, xh1_s), (kh0_s, kh1_s), (yh0_s, yh1_s)

    def lane_tile(c):
        return pl.ds(_aligned(c * LANES, LANES), LANES)

    def x_copies(s):
        rows = pl.ds(_aligned(s * TB, TB), TB)
        return [pltpu.make_async_copy(x_hbm.at[rows, lane_tile(c)],
                                      x_v.bitcast(BF16).at[c, rows, :], x_sem.at[s, c])
                for c in range(NT)]

    def w_copies(p):
        is_out = isinstance(p, int) and p == 3
        src = wo_hbm if is_out else wqkv_hbm
        return [pltpu.make_async_copy(src.at[:, lane_tile(c if is_out else p * NT + c)],
                                      w_v.bitcast(BF16).at[p, c], w_sem.at[p, c])
                for c in range(NT)]

    def tile_copies(c):
        cps = [pltpu.make_async_copy(h_hbm.at[lane_tile(c), pl.ds(jj * R * C, R * C)],
                                     h_v.bitcast(BF16).at[c, jj], t_sem.at[c, jj])
               for jj in range(NJ)]
        cps.append(pltpu.make_async_copy(k_hbm.at[:, lane_tile(c)],
                                         k_v.bitcast(BF16).at[c, pl.ds(16, S), :], t_sem.at[c, NJ]))
        cps.append(pltpu.make_async_copy(v_hbm.at[:, lane_tile(c)],
                                         v_v.bitcast(BF16).at[c], t_sem.at[c, NJ + 1]))
        return cps

    def out_copies(s):
        rows = pl.ds(_aligned(s * TB, TB), TB)
        return [pltpu.make_async_copy(out_v.bitcast(BF16).at[c, rows, :],
                                      out_hbm.at[rows, lane_tile(c)], out_sem.at[s, c])
                for c in range(NT)]

    def start(copies):
        for cp in copies:
            cp.start()

    def wait(copies):
        for cp in copies:
            cp.wait()

    def head_minor(j, d):
        return wt_s[j, pl.ds(d, H, stride=DH), :]

    def prep_wqkv(p):
        for j in range(NT):
            for c in range(NT):
                blk = _ld16(w_v.at[p, c], j * LANES, LANES)
                wt_s[j, pl.ds(c * LANES, LANES), :] = blk.T.astype(F32)
        for j in range(NT):
            for d in range(DH):
                _st16(wp_s.at[p, j], d * H, head_minor(j, d))

    def prep_wo():
        per = LANES // H
        for c in range(NT):
            wt_s[c] = _ld16(w_v.at[3, c], 0, D).astype(F32)
        for c in range(NT):
            for j in range(NT):
                blk = jnp.concatenate([head_minor(c, j * per + d) for d in range(per)], axis=0)
                _st16(wp_s.at[3, j], c * LANES, blk.astype(BF16).T)

    def dense_items(p, s, lhs_ref, dst):
        src = lhs_ref.at[:, pl.ds(_aligned(s * (TB // 2), TB // 2), TB // 2), :]
        last = NT - 1

        def head(c):
            def run():
                lhs = jnp.concatenate([_ld16(src.at[j], 0, TB) for j in range(last)], axis=1)
                w = jnp.concatenate([_ld16(wp_s.at[p, j], c * LANES, LANES)
                                     for j in range(last)], axis=1)
                dst[c] = jax.lax.dot_general(lhs, w, NT_DIMS, preferred_element_type=F32)
            return run

        def tail(c, r0, n):
            dst[c, pl.ds(r0, n), :] += jax.lax.dot_general(
                _ld16(src.at[last], r0, n), _ld16(wp_s.at[p, last], c * LANES, LANES),
                NT_DIMS, preferred_element_type=F32)

        def tails():
            for c in range(last):
                tail(c, 0, TB)

        def last_tail():
            for r0 in range(0, TB, TB // 4):
                tail(last, r0, TB // 4)

        return [head(c) for c in range(last)] + [tails, head(last), last_tail]

    def qkv_block(p, s):
        return qkv_s.at[p, :, pl.ds(_aligned(HALO + s * TB, 8), TB), :]

    def attn_items(t0, rows, o_ref, o_row0, first=False):
        scale = DH ** -0.5 * LOG2E
        win = qkv_s.at[:, :, pl.ds(_aligned(t0, 8), HALO + rows), :]
        dst = o_ref.at[:, pl.ds(_aligned((t0 - o_row0) // 2, 8), rows // 2), :]

        def item(r0):
            def run():
                q = [win[0, c, pl.ds(HALO + r0, AR), :] * scale for c in range(NT)]
                part = []
                for w in range(WIN):
                    taps = pl.ds(HALO + r0 - DIL * w, AR)
                    acc = q[0] * win[1, 0, taps, :]
                    for c in range(1, NT):
                        acc = acc + q[c] * win[1, c, taps, :]
                    part.append(acc)
                lane = jax.lax.broadcasted_iota(jnp.int32, (AR, LANES), 1)
                even = (lane & H) == 0
                logits = []
                for w in range(0, WIN, 2):
                    acc = (jnp.where(even, part[w], part[w + 1])
                           + pltpu.roll(jnp.where(even, part[w + 1], part[w]), H, 1))
                    acc = acc + pltpu.roll(acc, 2 * H, 1)
                    if first and r0 < DIL * (w + 1):
                        t = t0 + r0 + jax.lax.broadcasted_iota(jnp.int32, (AR, LANES), 0)
                        reach = jnp.where(even, DIL * w, DIL * (w + 1))
                        acc = jnp.where(t >= reach, acc, -1e9 * LOG2E)
                    logits.append(acc)
                m = logits[0]
                for l in logits[1:]:
                    m = jnp.maximum(m, l)
                m = jnp.maximum(m, pltpu.roll(m, H, 1))
                p = []
                for l in logits:
                    e = jnp.exp2(l - m)
                    other = pltpu.roll(e, H, 1)
                    p += [jnp.where(even, e, other), jnp.where(even, other, e)]
                den = p[0]
                for w in range(1, WIN):
                    den = den + p[w]
                inv = pltpu.reciprocal(den, full_range=False)
                for c in range(NT):
                    acc = p[0] * win[2, c, pl.ds(HALO + r0, AR), :]
                    for w in range(1, WIN):
                        acc = acc + p[w] * win[2, c, pl.ds(HALO + r0 - DIL * w, AR), :]
                    _st16(dst.at[c], r0, acc * inv)
            return run
        return [item(r0) for r0 in range(0, rows, AR)]

    def fwd_items(c, slot, jj):
        half = R * C // 2
        base = _aligned(jj * half, half)

        def dft(dst, tiles):
            parts = [jnp.dot(_ld16(f_ref, j * 2 * C, 2 * C), tile.astype(BF16),
                             preferred_element_type=F32) for j, tile in enumerate(tiles)]
            for k, spec in enumerate(_dft4(parts, -1)):
                dst[jj, k] = spec

        def h_item():
            for i in range(R):
                blk = pltpu.bitcast(h_v[c, jj, :, pl.ds(i * C, C)], BF16)
                ht_s[pl.ds(i * C // 2, C // 2), :] = pltpu.bitcast(blk.T, U32)
            words = [ht_s[pl.ds(j2, C, stride=2), :] for j2 in range(R // 2)]
            dft(kh_s[slot], [half_of(w) for w in words for half_of in (_lo, _hi)])

        def kv_item():
            taps = vec_s[c]
            kc = k_v.at[c, pl.ds(base, 8 + half), :]
            vc = v_v.at[c, pl.ds(base, half), :]
            kw = [kc[pl.ds(8 + o, C, stride=2), :] for o in (-2, -1, 0, 1)]
            ks = [_hi(kw[0]), _lo(kw[1]), _hi(kw[1]), _lo(kw[2]), _hi(kw[2]),
                  _lo(kw[3]), _hi(kw[3])]
            tiles = []
            for j in range(R):
                vw = vc[pl.ds(j // 2, C, stride=2), :]
                acc = ks[3 + j] * taps[0:1, :]
                for t in range(1, KS):
                    acc = acc + ks[3 + j - t] * taps[t:t + 1, :]
                tiles.append(acc * (_hi(vw) if j % 2 else _lo(vw)))
            dft(xh_s[slot], tiles)

        return [h_item, kv_item]

    def mac_items(c, slot, u):
        xh, kh, yh = xh_s[slot], kh_s[slot], yh_s[slot]

        def item(i, k):
            def run():
                r0 = _aligned(16 * (NJ * i + u), 16)
                re, im = pl.ds(r0, 8), pl.ds(r0 + 8, 8)
                x = [(xh[jj, k, re, :], xh[jj, k, im, :]) for jj in range(NJ)]
                h = [(kh[jj, k, re, :], kh[jj, k, im, :]) for jj in range(NJ)]
                fold = _cadd_i if i < 2 else _csub_i
                h = ([(h[0][0] + vec_s[c, KS:KS + 1, :], h[0][1])]
                     + [fold(h[m], h[m - 1]) for m in range(1, NJ)])
                for jj in range(NJ):
                    acc = _cmul(h[jj], x[0])
                    for j in range(1, jj + 1):
                        acc = _cadd(acc, _cmul(h[jj - j], x[j]))
                    yh[jj, k, re, :] = acc[0]
                    yh[jj, k, im, :] = acc[1]
            return run
        return [item(i, k) for i in range(C // 8 // NJ) for k in range(R)]

    def inv_items(c, slot, jj):
        def run():
            spec = _dft4([yh_s[slot][jj, k] for k in range(R)], +1)
            dst = y_s.at[c, pl.ds(_aligned(jj * R * C, R * C), R * C), :]
            for j in range(R):
                g = jnp.concatenate([_ld16(g_ref, 2 * j * C, C),
                                     _ld16(g_ref, (2 * j + 1) * C, C)], axis=1)
                dst[pl.ds(j, C, stride=R), :] = jnp.dot(g, spec[j].astype(BF16),
                                                        preferred_element_type=F32)
        return [run]

    def gate_items(t0, rows):
        src = x_v.at[:, pl.ds(_aligned(t0 // 2, 8), rows // 2), :]
        dst = gate_s.at[pl.ds(_aligned(t0, 8), rows), :]

        def item(r0):
            def run():
                z = _ld16(src.at[0], r0, AR).astype(F32) * vec_s[0, KS + 1:KS + 2, :]
                for c in range(1, NT):
                    z = z + _ld16(src.at[c], r0, AR).astype(F32) * vec_s[c, KS + 1:KS + 2, :]
                z = jnp.sum(z, axis=-1, keepdims=True)
                dst[pl.ds(r0, AR), :] = jnp.broadcast_to(1.0 / (1.0 + jnp.exp(-z)), (AR, LANES))
            return run
        return [item(r0) for r0 in range(0, rows, AR)]

    def mix_items(s):
        words = pl.ds(_aligned(s * (TB // 2), TB // 2), TB // 2)
        rows = pl.ds(_aligned(s * TB, TB), TB)
        x, out = x_v.at[:, words, :], out_v.at[:, words, :]
        att, y, gates = b_s.at[:, rows, :], y_s.at[:, rows, :], gate_s.at[rows, :]

        def item(r0):
            def run():
                gate = gates[pl.ds(r0, MR), :]
                for c in range(NT):
                    b = att[c, pl.ds(r0, MR), :]
                    a = _ld16(x.at[c], r0, MR).astype(F32) * y[c, pl.ds(r0, MR), :]
                    _st16(out.at[c], r0, gate * (a - b) + b)
            return run
        return [item(r0) for r0 in range(0, TB, MR)]

    def emit(*lists):
        for run in _interleave(*lists):
            run()

    start(w_copies(0) + x_copies(0))
    small = jnp.concatenate([sk_ref[...].astype(F32), d_ref[...].astype(F32).reshape(1, D),
                             gw_ref[...].astype(F32).reshape(1, D), jnp.zeros((2, D), F32)], axis=0)
    for c in range(NT):
        vec_s[c] = small[:, c * LANES:(c + 1) * LANES]
        k_v[c, pl.ds(0, 8), :] = jnp.zeros((8, LANES), U32)
    wait(w_copies(0))
    start(w_copies(1) + x_copies(1))
    prep_wqkv(0)
    wait(x_copies(0))
    start(w_copies(2))
    emit(dense_items(0, 0, x_v, qkv_block(0, 0)))
    wait(x_copies(1))
    start(tile_copies(0))

    @pl.loop(0, 2)
    def _(p):
        wait(w_copies(p + 1))
        emit(dense_items(p, 1 - p, x_v, qkv_block(p, 1 - p)), [lambda: prep_wqkv(p + 1)])

    start(x_copies(2) + x_copies(3) + w_copies(3))
    emit(dense_items(2, 0, x_v, qkv_block(2, 0)))
    for p in (1, 2):
        for c in range(NT):
            qkv_s[p, c, pl.ds(0, HALO), :] = jnp.broadcast_to(
                qkv_s[p, c, pl.ds(HALO, 1), :], (HALO, LANES))

    first_rows, tick_rows = TB // NJ, 80
    assert TB + (NT - 1) * NJ * tick_rows == O_SPLIT * TB and O_SPLIT * TB + NJ * tick_rows + 192 == S
    done = 4

    def stage_copy(i):
        return pltpu.make_async_copy(stage_s.at[i % STAGES], qkv_block((i + done) % 3, (i + done) // 3),
                                     stage_sem.at[i % STAGES])

    def tick(c, u, slot, mac, inv, first=False):
        i = c * NJ + u
        p, s = (i + done) % 3, (i + done) // 3

        @pl.when(i >= STAGES)
        def _():
            stage_copy(i - STAGES).wait()

        @pl.when(p == 0)
        def _():
            wait(x_copies(s))

            @pl.when(s + 2 < NB)
            def _():
                start(x_copies(s + 2))

        pl.when(u == 0)(lambda: wait(tile_copies(c)))
        pl.when(jnp.logical_and(u == 0, c + 1 < NT))(lambda: start(tile_copies(c + 1)))

        lists = [dense_items(p, s, x_v, stage_s.at[i % STAGES]), fwd_items(c, slot, u)]
        if inv:
            lists.append(inv_items(c - 2, slot, u))
        t0, rows = ((i * first_rows, first_rows) if first
                    else (TB + (i - NJ) * tick_rows, tick_rows))
        lists.append(attn_items(t0, rows, o0_s, 0, first))
        lists.append(gate_items(t0, rows))
        if mac:
            lists.append(mac_items(c - 1, 1 - slot, u))
        emit(*lists)
        stage_copy(i).start()

    def ticks(c, slot, **stages):
        pl.loop(0, NJ)(lambda u: tick(c, u, slot, **stages))

    ticks(0, 0, mac=False, inv=False, first=True)
    wait(w_copies(3))
    prep_wo()
    ticks(1, 1, mac=True, inv=False)

    @pl.loop(2, NT)
    def _(c):
        for slot in range(2):
            pl.when(c % 2 == slot)(lambda: ticks(c, slot, mac=True, inv=True))

    for i in range(NT * NJ - STAGES, NT * NJ):
        stage_copy(i).wait()

    def out_items(s, o_ref, o_block0):
        return dense_items(3, s - o_block0, o_ref, b_s.at[:, pl.ds(_aligned(s * TB, TB), TB), :])

    @pl.loop(0, NJ)
    def _(u):
        t0 = O_SPLIT * TB + u * tick_rows
        emit(out_items(u, o0_s, 0), inv_items(NT - 2, NT % 2, u),
             attn_items(t0, tick_rows, o1_s, O_SPLIT * TB), gate_items(t0, tick_rows),
             mac_items(NT - 1, (NT - 1) % 2, u))

    def mix(u):
        return mix_items(2 * u) + mix_items(2 * u + 1)

    done_rows = O_SPLIT * TB + NJ * tick_rows
    for u, rows in enumerate((64, 64, 64, 0)):
        s = NJ + u
        emit(out_items(s, o0_s, 0) if s < O_SPLIT else out_items(s, o1_s, O_SPLIT),
             inv_items(NT - 1, (NT - 1) % 2, u),
             attn_items(done_rows, rows, o1_s, O_SPLIT * TB) if rows else [],
             gate_items(done_rows, rows) if rows else [],
             mix(u - 1) if u else [])
        done_rows += rows
        if u:
            start(out_copies(2 * u - 2) + out_copies(2 * u - 1))
    for s in (NB - 2, NB - 1):
        emit(mix_items(s))
        start(out_copies(s))
    for s in range(NB):
        wait(out_copies(s))


@jax.jit
def pallas_gated_mix__ssm_conv_h3__sliding_local_dilated__prompt_kernel(
    A_q: jax.Array,
    A_k: jax.Array,
    A_v: jax.Array,
    A_shift_k: jax.Array,
    A_ssm_k: jax.Array,
    A_ssm_D: jax.Array,
    B_x: jax.Array,
    B_wqkv: jax.Array,
    B_wo: jax.Array,
    gate_w: jax.Array,
):
    del B_x
    fwd, inv = _dft_matrices()
    hbm = pl.BlockSpec(memory_space=pl.ANY)
    vmem = pl.BlockSpec(memory_space=pltpu.VMEM)
    out = pl.pallas_call(
        _kernel,
        out_shape=jax.ShapeDtypeStruct((S, D), A_q.dtype),
        in_specs=[hbm, hbm, hbm, vmem, hbm, vmem, hbm, hbm, vmem, vmem, vmem],
        out_specs=hbm,
        scratch_shapes=[
            pltpu.VMEM((NT, S // 2, LANES), U32),
            pltpu.VMEM((NT, 8 + S // 2, LANES), U32),
            pltpu.VMEM((NT, S // 2, LANES), U32),
            pltpu.VMEM((NT, NJ, LANES // 2, R * C), U32),
            pltpu.VMEM((4, NT, D // 2, LANES), U32),
            pltpu.VMEM((NT, S // 2, LANES), U32),
            pltpu.VMEM((NT, D, LANES), F32),
            pltpu.VMEM((4, NT, D // 2, LANES), U32),
            pltpu.VMEM((3, NT, HALO + S, LANES), F32),
            pltpu.VMEM((STAGES, NT, TB, LANES), F32),
            pltpu.VMEM((NT, O_SPLIT * TB // 2, LANES), U32),
            pltpu.VMEM((NT, (NB - O_SPLIT) * TB // 2, LANES), U32),
            pltpu.VMEM((NT, S, LANES), F32),
            pltpu.VMEM((R * C // 2, LANES), U32),
            *[pltpu.VMEM((NJ, R, 2 * C, LANES), F32)] * 6,
            pltpu.VMEM((NT, S, LANES), F32),
            pltpu.VMEM((S, LANES), F32),
            pltpu.VMEM((NT, 8, LANES), F32),
            pltpu.SemaphoreType.DMA((NB, NT)),
            pltpu.SemaphoreType.DMA((4, NT)),
            pltpu.SemaphoreType.DMA((NT, NJ + 2)),
            pltpu.SemaphoreType.DMA((STAGES,)),
            pltpu.SemaphoreType.DMA((NB, NT)),
        ],
        compiler_params=pltpu.CompilerParams(
            flags={'XLA_TPU_EVENLY_DISTRIBUTE_CRITICAL_NODES': True},
            vmem_limit_bytes=110 * 1024 * 1024),
    )(
        A_q.reshape(S, D), A_k.reshape(S, D), A_v.reshape(S, D),
        A_shift_k.T, A_ssm_k, A_ssm_D, B_wqkv, B_wo,
        gate_w, fwd, inv,
    )
    return out.reshape(A_q.shape)
```

```python
import numpy as np

import jax
import jax.numpy as jnp
import jax.experimental.pallas as pl
import jax.experimental.pallas.tpu as pltpu

S, D = 2048, 640
H, DH = 32, 20
WIN, DIL = 8, 2
KS = 4
LANES = 128
NT = D // LANES
C = 128
R = 4
NJ = S // (R * C)
TB = 256
NB = S // TB
HALO = 16
O_SPLIT = 6
STAGES = 3
MR = 32
AR = 16

LOG2E = float(np.log2(np.e))
F32 = jnp.float32
BF16 = jnp.bfloat16
U32 = jnp.uint32
NT_DIMS = (((1,), (1,)), ((), ()))


def _as_words(mat):
    bits = mat.astype(np.float32).astype(BF16).view(np.uint16).astype(np.uint32)
    return bits[0::2] | (bits[1::2] << 16)


def _dft_matrices():
    f = np.concatenate([np.arange(0, C, 2), np.arange(1, C, 2)]).astype(np.float64)
    theta = 2.0 * np.pi * (f + 0.5) / (2 * R * C)
    fwd, inv = [], []
    for j in range(R):
        ang = theta[:, None] * (R * np.arange(C, dtype=np.float64) + j)[None, :]
        mat = np.stack([np.cos(ang).reshape(C // 8, 8, C), -np.sin(ang).reshape(C // 8, 8, C)],
                       axis=1).reshape(2 * C, C)
        fwd.append(mat)
        inv += [mat[:C].T / (R * C), mat[C:].T / (R * C)]
    return _as_words(np.concatenate(fwd, axis=0)), _as_words(np.concatenate(inv, axis=0))


def _lo(words):
    return pltpu.bitcast(words << 16, F32)


def _hi(words):
    return pltpu.bitcast(words & np.uint32(0xFFFF0000), F32)


def _cadd(a, b):
    return a[0] + b[0], a[1] + b[1]


def _csub(a, b):
    return a[0] - b[0], a[1] - b[1]


def _cadd_i(a, b):
    return a[0] - b[1], a[1] + b[0]


def _csub_i(a, b):
    return a[0] + b[1], a[1] - b[0]


def _pairs(mat):
    return [(mat[r:r + 8], mat[r + 8:r + 16]) for r in range(0, mat.shape[0], 16)]


def _dft4(mats, sign):
    plus, minus = (_cadd_i, _csub_i) if sign > 0 else (_csub_i, _cadd_i)
    out = [[] for _ in mats]
    for e in zip(*map(_pairs, mats)):
        a, b = _cadd(e[0], e[2]), _csub(e[0], e[2])
        c, d = _cadd(e[1], e[3]), _csub(e[1], e[3])
        for rows, val in zip(out, (_cadd(a, c), plus(b, d), _csub(a, c), minus(b, d))):
            rows.extend(val)
    return [jnp.concatenate(rows, axis=0) for rows in out]


def _cmul(a, b):
    return a[0] * b[0] - a[1] * b[1], a[0] * b[1] + a[1] * b[0]


def _ld16(ref, r0, n):
    return pltpu.bitcast(ref[pl.ds(r0 // 2, n // 2), :], BF16)


def _st16(ref, r0, value):
    ref[pl.ds(r0 // 2, value.shape[0] // 2), :] = pltpu.bitcast(value.astype(BF16), U32)


def _interleave(*lists):
    keyed = []
    for li, items in enumerate(lists):
        for i, item in enumerate(items):
            keyed.append(((i + 0.5) / len(items), li, i, item))
    keyed.sort(key=lambda t: t[:3])
    return [t[3] for t in keyed]


def _aligned(index, multiple):
    return index if isinstance(index, int) else pl.multiple_of(index, multiple)


def _kernel(x_hbm, k_hbm, v_hbm, sk_ref, h_hbm, d_ref, wqkv_hbm, wo_hbm, gw_ref,
            f_ref, g_ref, out_hbm,
            x_v, k_v, v_v, h_v, w_v, out_v, wt_s, wp_s, qkv_s, stage_s, o0_s, o1_s, b_s, ht_s,
            xh0_s, xh1_s, kh0_s, kh1_s, yh0_s, yh1_s, y_s, gate_s, vec_s,
            x_sem, w_sem, t_sem, stage_sem, out_sem):
    xh_s, kh_s, yh_s = (xh0_s, xh1_s), (kh0_s, kh1_s), (yh0_s, yh1_s)

    def lane_tile(c):
        return pl.ds(_aligned(c * LANES, LANES), LANES)

    def x_copies(s):
        rows = pl.ds(_aligned(s * TB, TB), TB)
        return [pltpu.make_async_copy(x_hbm.at[rows, lane_tile(c)],
                                      x_v.bitcast(BF16).at[c, rows, :], x_sem.at[s, c])
                for c in range(NT)]

    def w_copies(p):
        is_out = isinstance(p, int) and p == 3
        src = wo_hbm if is_out else wqkv_hbm
        return [pltpu.make_async_copy(src.at[:, lane_tile(c if is_out else p * NT + c)],
                                      w_v.bitcast(BF16).at[p, c], w_sem.at[p, c])
                for c in range(NT)]

    def tile_copies(c):
        cps = [pltpu.make_async_copy(h_hbm.at[lane_tile(c), pl.ds(jj * R * C, R * C)],
                                     h_v.bitcast(BF16).at[c, jj], t_sem.at[c, jj])
               for jj in range(NJ)]
        cps.append(pltpu.make_async_copy(k_hbm.at[:, lane_tile(c)],
                                         k_v.bitcast(BF16).at[c, pl.ds(16, S), :], t_sem.at[c, NJ]))
        cps.append(pltpu.make_async_copy(v_hbm.at[:, lane_tile(c)],
                                         v_v.bitcast(BF16).at[c], t_sem.at[c, NJ + 1]))
        return cps

    def out_copies(s):
        rows = pl.ds(_aligned(s * TB, TB), TB)
        return [pltpu.make_async_copy(out_v.bitcast(BF16).at[c, rows, :],
                                      out_hbm.at[rows, lane_tile(c)], out_sem.at[s, c])
                for c in range(NT)]

    def start(copies):
        for cp in copies:
            cp.start()

    def wait(copies):
        for cp in copies:
            cp.wait()

    def head_minor(j, d):
        return wt_s[j, pl.ds(d, H, stride=DH), :]

    def prep_wqkv(p, arrived=lambda c: None):
        for c in range(NT):
            arrived(c)
            for j in range(NT):
                blk = _ld16(w_v.at[p, c], j * LANES, LANES)
                wt_s[j, pl.ds(c * LANES, LANES), :] = blk.T.astype(F32)
        for j in range(NT):
            for d in range(DH):
                _st16(wp_s.at[p, j], d * H, head_minor(j, d))

    def prep_wo():
        per = LANES // H
        for c in range(NT):
            wt_s[c] = _ld16(w_v.at[3, c], 0, D).astype(F32)
        for c in range(NT):
            for j in range(NT):
                blk = jnp.concatenate([head_minor(c, j * per + d) for d in range(per)], axis=0)
                _st16(wp_s.at[3, j], c * LANES, blk.astype(BF16).T)

    def dense_items(p, s, lhs_ref, dst):
        src = lhs_ref.at[:, pl.ds(_aligned(s * (TB // 2), TB // 2), TB // 2), :]
        last = NT - 1

        def head(c):
            def run():
                lhs = jnp.concatenate([_ld16(src.at[j], 0, TB) for j in range(last)], axis=1)
                w = jnp.concatenate([_ld16(wp_s.at[p, j], c * LANES, LANES)
                                     for j in range(last)], axis=1)
                dst[c] = jax.lax.dot_general(lhs, w, NT_DIMS, preferred_element_type=F32)
            return run

        def tail(c, r0, n):
            dst[c, pl.ds(r0, n), :] += jax.lax.dot_general(
                _ld16(src.at[last], r0, n), _ld16(wp_s.at[p, last], c * LANES, LANES),
                NT_DIMS, preferred_element_type=F32)

        def tails():
            for c in range(last):
                tail(c, 0, TB)

        def last_tail():
            for r0 in range(0, TB, TB // 4):
                tail(last, r0, TB // 4)

        return [head(c) for c in range(last)] + [tails, head(last), last_tail]

    def qkv_block(p, s):
        return qkv_s.at[p, :, pl.ds(_aligned(HALO + s * TB, 8), TB), :]

    def attn_items(t0, rows, o_ref, o_row0, first=False):
        scale = DH ** -0.5 * LOG2E
        win = qkv_s.at[:, :, pl.ds(_aligned(t0, 8), HALO + rows), :]
        dst = o_ref.at[:, pl.ds(_aligned((t0 - o_row0) // 2, 8), rows // 2), :]

        def item(r0):
            def run():
                q = [win[0, c, pl.ds(HALO + r0, AR), :] * scale for c in range(NT)]
                part = []
                for w in range(WIN):
                    taps = pl.ds(HALO + r0 - DIL * w, AR)
                    acc = q[0] * win[1, 0, taps, :]
                    for c in range(1, NT):
                        acc = acc + q[c] * win[1, c, taps, :]
                    part.append(acc)
                lane = jax.lax.broadcasted_iota(jnp.int32, (AR, LANES), 1)
                even = (lane & H) == 0
                logits = []
                for w in range(0, WIN, 2):
                    acc = (jnp.where(even, part[w], part[w + 1])
                           + pltpu.roll(jnp.where(even, part[w + 1], part[w]), H, 1))
                    acc = acc + pltpu.roll(acc, 2 * H, 1)
                    if first and r0 < DIL * (w + 1):
                        t = t0 + r0 + jax.lax.broadcasted_iota(jnp.int32, (AR, LANES), 0)
                        reach = jnp.where(even, DIL * w, DIL * (w + 1))
                        acc = jnp.where(t >= reach, acc, -1e9 * LOG2E)
                    logits.append(acc)
                m = logits[0]
                for l in logits[1:]:
                    m = jnp.maximum(m, l)
                m = jnp.maximum(m, pltpu.roll(m, H, 1))
                p = []
                for l in logits:
                    e = jnp.exp2(l - m)
                    other = pltpu.roll(e, H, 1)
                    p += [jnp.where(even, e, other), jnp.where(even, other, e)]
                den = p[0]
                for w in range(1, WIN):
                    den = den + p[w]
                inv = pltpu.reciprocal(den, full_range=False)
                for c in range(NT):
                    acc = p[0] * win[2, c, pl.ds(HALO + r0, AR), :]
                    for w in range(1, WIN):
                        acc = acc + p[w] * win[2, c, pl.ds(HALO + r0 - DIL * w, AR), :]
                    _st16(dst.at[c], r0, acc * inv)
            return run
        return [item(r0) for r0 in range(0, rows, AR)]

    def fwd_items(c, slot, jj):
        half = R * C // 2
        base = _aligned(jj * half, half)

        def dft(dst, tiles):
            parts = [jnp.dot(_ld16(f_ref, j * 2 * C, 2 * C), tile.astype(BF16),
                             preferred_element_type=F32) for j, tile in enumerate(tiles)]
            for k, spec in enumerate(_dft4(parts, -1)):
                dst[jj, k] = spec

        def h_item():
            for i in range(R):
                blk = pltpu.bitcast(h_v[c, jj, :, pl.ds(i * C, C)], BF16)
                ht_s[pl.ds(i * C // 2, C // 2), :] = pltpu.bitcast(blk.T, U32)
            words = [ht_s[pl.ds(j2, C, stride=2), :] for j2 in range(R // 2)]
            dft(kh_s[slot], [half_of(w) for w in words for half_of in (_lo, _hi)])

        def kv_item():
            taps = vec_s[c]
            kc = k_v.at[c, pl.ds(base, 8 + half), :]
            vc = v_v.at[c, pl.ds(base, half), :]
            kw = [kc[pl.ds(8 + o, C, stride=2), :] for o in (-2, -1, 0, 1)]
            ks = [_hi(kw[0]), _lo(kw[1]), _hi(kw[1]), _lo(kw[2]), _hi(kw[2]),
                  _lo(kw[3]), _hi(kw[3])]
            tiles = []
            for j in range(R):
                vw = vc[pl.ds(j // 2, C, stride=2), :]
                acc = ks[3 + j] * taps[0:1, :]
                for t in range(1, KS):
                    acc = acc + ks[3 + j - t] * taps[t:t + 1, :]
                tiles.append(acc * (_hi(vw) if j % 2 else _lo(vw)))
            dft(xh_s[slot], tiles)

        return [h_item, kv_item]

    def mac_items(c, slot, u):
        xh, kh, yh = xh_s[slot], kh_s[slot], yh_s[slot]

        def item(i, k):
            def run():
                r0 = _aligned(16 * (NJ * i + u), 16)
                re, im = pl.ds(r0, 8), pl.ds(r0 + 8, 8)
                x = [(xh[jj, k, re, :], xh[jj, k, im, :]) for jj in range(NJ)]
                h = [(kh[jj, k, re, :], kh[jj, k, im, :]) for jj in range(NJ)]
                fold = _cadd_i if i < 2 else _csub_i
                h = ([(h[0][0] + vec_s[c, KS:KS + 1, :], h[0][1])]
                     + [fold(h[m], h[m - 1]) for m in range(1, NJ)])
                for jj in range(NJ):
                    acc = _cmul(h[jj], x[0])
                    for j in range(1, jj + 1):
                        acc = _cadd(acc, _cmul(h[jj - j], x[j]))
                    yh[jj, k, re, :] = acc[0]
                    yh[jj, k, im, :] = acc[1]
            return run
        return [item(i, k) for i in range(C // 8 // NJ) for k in range(R)]

    def inv_items(c, slot, jj):
        def run():
            spec = _dft4([yh_s[slot][jj, k] for k in range(R)], +1)
            dst = y_s.at[c, pl.ds(_aligned(jj * R * C, R * C), R * C), :]
            for j in range(R):
                g = jnp.concatenate([_ld16(g_ref, 2 * j * C, C),
                                     _ld16(g_ref, (2 * j + 1) * C, C)], axis=1)
                dst[pl.ds(j, C, stride=R), :] = jnp.dot(g, spec[j].astype(BF16),
                                                        preferred_element_type=F32)
        return [run]

    def gate_items(t0, rows):
        src = x_v.at[:, pl.ds(_aligned(t0 // 2, 8), rows // 2), :]
        dst = gate_s.at[pl.ds(_aligned(t0, 8), rows), :]

        def item(r0):
            def run():
                z = _ld16(src.at[0], r0, AR).astype(F32) * vec_s[0, KS + 1:KS + 2, :]
                for c in range(1, NT):
                    z = z + _ld16(src.at[c], r0, AR).astype(F32) * vec_s[c, KS + 1:KS + 2, :]
                z = jnp.sum(z, axis=-1, keepdims=True)
                dst[pl.ds(r0, AR), :] = jnp.broadcast_to(1.0 / (1.0 + jnp.exp(-z)), (AR, LANES))
            return run
        return [item(r0) for r0 in range(0, rows, AR)]

    def mix_items(s):
        words = pl.ds(_aligned(s * (TB // 2), TB // 2), TB // 2)
        rows = pl.ds(_aligned(s * TB, TB), TB)
        x, out = x_v.at[:, words, :], out_v.at[:, words, :]
        att, y, gates = b_s.at[:, rows, :], y_s.at[:, rows, :], gate_s.at[rows, :]

        def item(r0):
            def run():
                gate = gates[pl.ds(r0, MR), :]
                for c in range(NT):
                    b = att[c, pl.ds(r0, MR), :]
                    a = _ld16(x.at[c], r0, MR).astype(F32) * y[c, pl.ds(r0, MR), :]
                    _st16(out.at[c], r0, gate * (a - b) + b)
            return run
        return [item(r0) for r0 in range(0, TB, MR)]

    def emit(*lists):
        for run in _interleave(*lists):
            run()

    start(w_copies(0) + x_copies(0))
    small = jnp.concatenate([sk_ref[...].astype(F32), d_ref[...].astype(F32).reshape(1, D),
                             gw_ref[...].astype(F32).reshape(1, D), jnp.zeros((2, D), F32)], axis=0)
    for c in range(NT):
        vec_s[c] = small[:, c * LANES:(c + 1) * LANES]
        k_v[c, pl.ds(0, 8), :] = jnp.zeros((8, LANES), U32)

    def first_weights(c):
        wait(w_copies(0)[c:c + 1])
        if c == 0:
            start(w_copies(1) + x_copies(1))

    prep_wqkv(0, first_weights)
    wait(x_copies(0))
    start(w_copies(2))
    emit(dense_items(0, 0, x_v, qkv_block(0, 0)))
    wait(x_copies(1))
    start(tile_copies(0))

    @pl.loop(0, 2)
    def _(p):
        wait(w_copies(p + 1))
        emit(dense_items(p, 1 - p, x_v, qkv_block(p, 1 - p)), [lambda: prep_wqkv(p + 1)])

    start(x_copies(2) + x_copies(3) + w_copies(3))
    emit(dense_items(2, 0, x_v, qkv_block(2, 0)))
    for p in (1, 2):
        for c in range(NT):
            qkv_s[p, c, pl.ds(0, HALO), :] = jnp.broadcast_to(
                qkv_s[p, c, pl.ds(HALO, 1), :], (HALO, LANES))

    first_rows, tick_rows = TB // NJ, 80
    assert TB + (NT - 1) * NJ * tick_rows == O_SPLIT * TB
    done = 4

    def stage_copy(i):
        return pltpu.make_async_copy(stage_s.at[i % STAGES], qkv_block((i + done) % 3, (i + done) // 3),
                                     stage_sem.at[i % STAGES])

    def tick(c, u, slot, mac, inv, first=False):
        i = c * NJ + u
        p, s = (i + done) % 3, (i + done) // 3

        @pl.when(i >= STAGES)
        def _():
            stage_copy(i - STAGES).wait()

        @pl.when(p == 0)
        def _():
            wait(x_copies(s))

            @pl.when(s + 2 < NB)
            def _():
                start(x_copies(s + 2))

        pl.when(u == 0)(lambda: wait(tile_copies(c)))
        pl.when(jnp.logical_and(u == 0, c + 1 < NT))(lambda: start(tile_copies(c + 1)))

        lists = [dense_items(p, s, x_v, stage_s.at[i % STAGES]), fwd_items(c, slot, u)]
        if inv:
            lists.append(inv_items(c - 2, slot, u))
        t0, rows = ((i * first_rows, first_rows) if first
                    else (TB + (i - NJ) * tick_rows, tick_rows))
        lists.append(attn_items(t0, rows, o0_s, 0, first))
        lists.append(gate_items(t0, rows))
        if mac:
            lists.append(mac_items(c - 1, 1 - slot, u))
        emit(*lists)
        stage_copy(i).start()

    def ticks(c, slot, **stages):
        pl.loop(0, NJ)(lambda u: tick(c, u, slot, **stages))

    ticks(0, 0, mac=False, inv=False, first=True)
    wait(w_copies(3))
    prep_wo()
    ticks(1, 1, mac=True, inv=False)

    @pl.loop(2, NT)
    def _(c):
        for slot in range(2):
            pl.when(c % 2 == slot)(lambda: ticks(c, slot, mac=True, inv=True))

    for i in range(NT * NJ - STAGES, NT * NJ):
        stage_copy(i).wait()

    def out_items(s, o_ref, o_block0):
        return dense_items(3, s - o_block0, o_ref, b_s.at[:, pl.ds(_aligned(s * TB, TB), TB), :])

    @pl.loop(0, NJ)
    def _(u):
        t0 = O_SPLIT * TB + u * tick_rows
        emit(out_items(u, o0_s, 0), inv_items(NT - 2, NT % 2, u),
             attn_items(t0, tick_rows, o1_s, O_SPLIT * TB), gate_items(t0, tick_rows),
             mac_items(NT - 1, (NT - 1) % 2, u))

    done_rows = O_SPLIT * TB + NJ * tick_rows
    for s, rows, chunks, mixed in ((4, 64, (0, 1), ()), (5, 64, (2,), (0, 1, 2)),
                                   (6, 64, (3,), (3, 4)), (7, 0, (), (5, 6))):
        emit(out_items(s, o0_s, 0) if s < O_SPLIT else out_items(s, o1_s, O_SPLIT),
             [it for jj in chunks for it in inv_items(NT - 1, (NT - 1) % 2, jj)],
             attn_items(done_rows, rows, o1_s, O_SPLIT * TB) if rows else [],
             gate_items(done_rows, rows) if rows else [],
             [it for m in mixed for it in mix_items(m)])
        done_rows += rows
        for m in mixed:
            start(out_copies(m))
    assert done_rows == S
    emit(mix_items(NB - 1))
    start(out_copies(NB - 1))
    for s in range(NB):
        wait(out_copies(s))


@jax.jit
def pallas_gated_mix__ssm_conv_h3__sliding_local_dilated__prompt_kernel(
    A_q: jax.Array,
    A_k: jax.Array,
    A_v: jax.Array,
    A_shift_k: jax.Array,
    A_ssm_k: jax.Array,
    A_ssm_D: jax.Array,
    B_x: jax.Array,
    B_wqkv: jax.Array,
    B_wo: jax.Array,
    gate_w: jax.Array,
):
    del B_x
    fwd, inv = _dft_matrices()
    hbm = pl.BlockSpec(memory_space=pl.ANY)
    vmem = pl.BlockSpec(memory_space=pltpu.VMEM)
    out = pl.pallas_call(
        _kernel,
        out_shape=jax.ShapeDtypeStruct((S, D), A_q.dtype),
        in_specs=[hbm, hbm, hbm, vmem, hbm, vmem, hbm, hbm, vmem, vmem, vmem],
        out_specs=hbm,
        scratch_shapes=[
            pltpu.VMEM((NT, S // 2, LANES), U32),
            pltpu.VMEM((NT, 8 + S // 2, LANES), U32),
            pltpu.VMEM((NT, S // 2, LANES), U32),
            pltpu.VMEM((NT, NJ, LANES // 2, R * C), U32),
            pltpu.VMEM((4, NT, D // 2, LANES), U32),
            pltpu.VMEM((NT, S // 2, LANES), U32),
            pltpu.VMEM((NT, D, LANES), F32),
            pltpu.VMEM((4, NT, D // 2, LANES), U32),
            pltpu.VMEM((3, NT, HALO + S, LANES), F32),
            pltpu.VMEM((STAGES, NT, TB, LANES), F32),
            pltpu.VMEM((NT, O_SPLIT * TB // 2, LANES), U32),
            pltpu.VMEM((NT, (NB - O_SPLIT) * TB // 2, LANES), U32),
            pltpu.VMEM((NT, S, LANES), F32),
            pltpu.VMEM((R * C // 2, LANES), U32),
            *[pltpu.VMEM((NJ, R, 2 * C, LANES), F32)] * 6,
            pltpu.VMEM((NT, S, LANES), F32),
            pltpu.VMEM((S, LANES), F32),
            pltpu.VMEM((NT, 8, LANES), F32),
            pltpu.SemaphoreType.DMA((NB, NT)),
            pltpu.SemaphoreType.DMA((4, NT)),
            pltpu.SemaphoreType.DMA((NT, NJ + 2)),
            pltpu.SemaphoreType.DMA((STAGES,)),
            pltpu.SemaphoreType.DMA((NB, NT)),
        ],
        compiler_params=pltpu.CompilerParams(
            flags={'XLA_TPU_EVENLY_DISTRIBUTE_CRITICAL_NODES': True},
            vmem_limit_bytes=110 * 1024 * 1024),
    )(
        A_q.reshape(S, D), A_k.reshape(S, D), A_v.reshape(S, D),
        A_shift_k.T, A_ssm_k, A_ssm_D, B_wqkv, B_wo,
        gate_w, fwd, inv,
    )
    return out.reshape(A_q.shape)
```

```python
import numpy as np

import jax
import jax.numpy as jnp
import jax.experimental.pallas as pl
import jax.experimental.pallas.tpu as pltpu

S, D = 2048, 640
H, DH = 32, 20
WIN, DIL = 8, 2
KS = 4
LANES = 128
NT = D // LANES
C = 128
R = 4
NJ = S // (R * C)
TB = 256
NB = S // TB
HALO = 16
O_SPLIT = 6
STAGES = 3
SPARE = 24
MR = 32
AR = 16

LOG2E = float(np.log2(np.e))
F32 = jnp.float32
BF16 = jnp.bfloat16
U32 = jnp.uint32
NT_DIMS = (((1,), (1,)), ((), ()))


def _as_words(mat):
    bits = mat.astype(np.float32).astype(BF16).view(np.uint16).astype(np.uint32)
    return bits[0::2] | (bits[1::2] << 16)


def _dft_matrices():
    f = np.concatenate([np.arange(0, C, 2), np.arange(1, C, 2)]).astype(np.float64)
    theta = 2.0 * np.pi * (f + 0.5) / (2 * R * C)
    fwd, inv = [], []
    for j in range(R):
        ang = theta[:, None] * (R * np.arange(C, dtype=np.float64) + j)[None, :]
        mat = np.stack([np.cos(ang).reshape(C // 8, 8, C), -np.sin(ang).reshape(C // 8, 8, C)],
                       axis=1).reshape(2 * C, C)
        fwd.append(mat)
        inv += [mat[:C].T / (R * C), mat[C:].T / (R * C)]
    return _as_words(np.concatenate(fwd, axis=0)), _as_words(np.concatenate(inv, axis=0))


def _lo(words):
    return pltpu.bitcast(words << 16, F32)


def _hi(words):
    return pltpu.bitcast(words & np.uint32(0xFFFF0000), F32)


def _cadd(a, b):
    return a[0] + b[0], a[1] + b[1]


def _csub(a, b):
    return a[0] - b[0], a[1] - b[1]


def _cadd_i(a, b):
    return a[0] - b[1], a[1] + b[0]


def _csub_i(a, b):
    return a[0] + b[1], a[1] - b[0]


def _pairs(mat):
    return [(mat[r:r + 8], mat[r + 8:r + 16]) for r in range(0, mat.shape[0], 16)]


def _dft4(mats, sign):
    plus, minus = (_cadd_i, _csub_i) if sign > 0 else (_csub_i, _cadd_i)
    out = [[] for _ in mats]
    for e in zip(*map(_pairs, mats)):
        a, b = _cadd(e[0], e[2]), _csub(e[0], e[2])
        c, d = _cadd(e[1], e[3]), _csub(e[1], e[3])
        for rows, val in zip(out, (_cadd(a, c), plus(b, d), _csub(a, c), minus(b, d))):
            rows.extend(val)
    return [jnp.concatenate(rows, axis=0) for rows in out]


def _cmul(a, b):
    return a[0] * b[0] - a[1] * b[1], a[0] * b[1] + a[1] * b[0]


def _ld16(ref, r0, n):
    return pltpu.bitcast(ref[pl.ds(r0 // 2, n // 2), :], BF16)


def _st16(ref, r0, value):
    ref[pl.ds(r0 // 2, value.shape[0] // 2), :] = pltpu.bitcast(value.astype(BF16), U32)


def _interleave(*lists):
    keyed = []
    for li, items in enumerate(lists):
        for i, item in enumerate(items):
            keyed.append(((i + 0.5) / len(items), li, i, item))
    keyed.sort(key=lambda t: t[:3])
    return [t[3] for t in keyed]


def _aligned(index, multiple):
    return index if isinstance(index, int) else pl.multiple_of(index, multiple)


def _kernel(x_hbm, k_hbm, v_hbm, sk_ref, h_hbm, d_ref, wqkv_hbm, wo_hbm, gw_ref,
            f_ref, g_ref, out_hbm,
            x_v, k_v, v_v, h_v, w_v, out_v, wt_s, wp_s, qkv_s, stage_s, o0_s, o1_s, b_s, ht_s,
            xh0_s, xh1_s, kh0_s, kh1_s, yh0_s, yh1_s, y_s, gate_s, vec_s,
            x_sem, w_sem, t_sem, stage_sem, out_sem):
    xh_s, kh_s, yh_s = (xh0_s, xh1_s), (kh0_s, kh1_s), (yh0_s, yh1_s)

    def lane_tile(c):
        return pl.ds(_aligned(c * LANES, LANES), LANES)

    def x_copies(s):
        rows = pl.ds(_aligned(s * TB, TB), TB)
        return [pltpu.make_async_copy(x_hbm.at[rows, lane_tile(c)],
                                      x_v.bitcast(BF16).at[c, rows, :], x_sem.at[s, c])
                for c in range(NT)]

    def w_copies(p, tiles=range(NT)):
        is_out = isinstance(p, int) and p == 3
        src = wo_hbm if is_out else wqkv_hbm
        return [pltpu.make_async_copy(src.at[:, lane_tile(c if is_out else p * NT + c)],
                                      w_v.bitcast(BF16).at[p, c], w_sem.at[p, c])
                for c in tiles]

    def tile_copies(c):
        cps = [pltpu.make_async_copy(h_hbm.at[lane_tile(c), pl.ds(jj * R * C, R * C)],
                                     h_v.bitcast(BF16).at[c, jj], t_sem.at[c, jj])
               for jj in range(NJ)]
        cps.append(pltpu.make_async_copy(k_hbm.at[:, lane_tile(c)],
                                         k_v.bitcast(BF16).at[c, pl.ds(16, S), :], t_sem.at[c, NJ]))
        cps.append(pltpu.make_async_copy(v_hbm.at[:, lane_tile(c)],
                                         v_v.bitcast(BF16).at[c, pl.ds(0, S), :], t_sem.at[c, NJ + 1]))
        return cps

    def out_copies(s):
        rows = pl.ds(_aligned(s * TB, TB), TB)
        return [pltpu.make_async_copy(out_v.bitcast(BF16).at[c, rows, :],
                                      out_hbm.at[rows, lane_tile(c)], out_sem.at[s, c])
                for c in range(NT)]

    def start(copies):
        for cp in copies:
            cp.start()

    def wait(copies):
        for cp in copies:
            cp.wait()

    def head_minor(j, d):
        return wt_s[j, pl.ds(d, H, stride=DH), :]

    def prep_wqkv(p, arrived=lambda c: None):
        for c in range(NT):
            arrived(c)
            for j in range(NT):
                blk = _ld16(w_v.at[p, c], j * LANES, LANES)
                wt_s[j, pl.ds(c * LANES, LANES), :] = blk.T.astype(F32)
        for j in range(NT):
            for d in range(DH):
                _st16(wp_s.at[p, j], d * H, head_minor(j, d))

    def prep_wo():
        per = LANES // H
        for c in range(NT):
            wt_s[c, pl.ds(0, D), :] = _ld16(w_v.at[3, c], 0, D).astype(F32)
        for c in range(NT):
            for j in range(NT):
                blk = jnp.concatenate([head_minor(c, j * per + d) for d in range(per)], axis=0)
                _st16(wp_s.at[3, j], c * LANES, blk.astype(BF16).T)

    def dense_items(p, s, lhs_ref, dst):
        src = lhs_ref.at[:, pl.ds(_aligned(s * (TB // 2), TB // 2), TB // 2), :]
        last = NT - 1

        def head(c):
            def run():
                lhs = jnp.concatenate([_ld16(src.at[j], 0, TB) for j in range(last)], axis=1)
                w = jnp.concatenate([_ld16(wp_s.at[p, j], c * LANES, LANES)
                                     for j in range(last)], axis=1)
                dst[c] = jax.lax.dot_general(lhs, w, NT_DIMS, preferred_element_type=F32)
            return run

        def tail(c, r0, n):
            dst[c, pl.ds(r0, n), :] += jax.lax.dot_general(
                _ld16(src.at[last], r0, n), _ld16(wp_s.at[p, last], c * LANES, LANES),
                NT_DIMS, preferred_element_type=F32)

        def tails():
            for c in range(last):
                tail(c, 0, TB)

        def last_tail():
            for r0 in range(0, TB, TB // 4):
                tail(last, r0, TB // 4)

        return [head(c) for c in range(last)] + [tails, head(last), last_tail]

    def qkv_block(p, s):
        return qkv_s.at[p, :, pl.ds(_aligned(HALO + s * TB, 8), TB), :]

    def attn_items(t0, rows, o_ref, o_row0, first=False):
        scale = DH ** -0.5 * LOG2E
        win = qkv_s.at[:, :, pl.ds(_aligned(t0, 8), HALO + rows), :]
        dst = o_ref.at[:, pl.ds(_aligned((t0 - o_row0) // 2, 8), rows // 2), :]

        def item(r0):
            def run():
                q = [win[0, c, pl.ds(HALO + r0, AR), :] * scale for c in range(NT)]
                part = []
                for w in range(WIN):
                    taps = pl.ds(HALO + r0 - DIL * w, AR)
                    acc = q[0] * win[1, 0, taps, :]
                    for c in range(1, NT):
                        acc = acc + q[c] * win[1, c, taps, :]
                    part.append(acc)
                lane = jax.lax.broadcasted_iota(jnp.int32, (AR, LANES), 1)
                even = (lane & H) == 0
                logits = []
                for w in range(0, WIN, 2):
                    acc = (jnp.where(even, part[w], part[w + 1])
                           + pltpu.roll(jnp.where(even, part[w + 1], part[w]), H, 1))
                    acc = acc + pltpu.roll(acc, 2 * H, 1)
                    if first and r0 < DIL * (w + 1):
                        t = t0 + r0 + jax.lax.broadcasted_iota(jnp.int32, (AR, LANES), 0)
                        reach = jnp.where(even, DIL * w, DIL * (w + 1))
                        acc = jnp.where(t >= reach, acc, -1e9 * LOG2E)
                    logits.append(acc)
                m = logits[0]
                for l in logits[1:]:
                    m = jnp.maximum(m, l)
                m = jnp.maximum(m, pltpu.roll(m, H, 1))
                p = []
                for l in logits:
                    e = jnp.exp2(l - m)
                    other = pltpu.roll(e, H, 1)
                    p += [jnp.where(even, e, other), jnp.where(even, other, e)]
                den = p[0]
                for w in range(1, WIN):
                    den = den + p[w]
                inv = pltpu.reciprocal(den, full_range=False)
                for c in range(NT):
                    acc = p[0] * win[2, c, pl.ds(HALO + r0, AR), :]
                    for w in range(1, WIN):
                        acc = acc + p[w] * win[2, c, pl.ds(HALO + r0 - DIL * w, AR), :]
                    _st16(dst.at[c], r0, acc * inv)
            return run
        return [item(r0) for r0 in range(0, rows, AR)]

    def fwd_items(c, slot, jj):
        half = R * C // 2
        base = _aligned(jj * half, half)

        def dft(dst, tiles):
            parts = [jnp.dot(_ld16(f_ref, j * 2 * C, 2 * C), tile.astype(BF16),
                             preferred_element_type=F32) for j, tile in enumerate(tiles)]
            for k, spec in enumerate(_dft4(parts, -1)):
                dst[jj, k] = spec

        def h_item():
            for i in range(R):
                blk = pltpu.bitcast(h_v[c, jj, :, pl.ds(i * C, C)], BF16)
                ht_s[pl.ds(i * C // 2, C // 2), :] = pltpu.bitcast(blk.T, U32)
            words = [ht_s[pl.ds(j2, C, stride=2), :] for j2 in range(R // 2)]
            dft(kh_s[slot], [half_of(w) for w in words for half_of in (_lo, _hi)])

        def kv_item():
            taps = vec_s[c]
            kc = k_v.at[c, pl.ds(base, 8 + half + SPARE), :]
            vc = v_v.at[c, pl.ds(base, half + SPARE), :]
            kw = [kc[pl.ds(8 + o, C, stride=2), :] for o in (-2, -1, 0, 1)]
            ks = [_hi(kw[0]), _lo(kw[1]), _hi(kw[1]), _lo(kw[2]), _hi(kw[2]),
                  _lo(kw[3]), _hi(kw[3])]
            tiles = []
            for j in range(R):
                vw = vc[pl.ds(j // 2, C, stride=2), :]
                acc = ks[3 + j] * taps[0:1, :]
                for t in range(1, KS):
                    acc = acc + ks[3 + j - t] * taps[t:t + 1, :]
                tiles.append(acc * (_hi(vw) if j % 2 else _lo(vw)))
            dft(xh_s[slot], tiles)

        return [h_item, kv_item]

    def mac_items(c, slot, u):
        xh, kh, yh = xh_s[slot], kh_s[slot], yh_s[slot]

        def item(i, k):
            def run():
                r0 = _aligned(16 * (NJ * i + u), 16)
                re, im = pl.ds(r0, 8), pl.ds(r0 + 8, 8)
                x = [(xh[jj, k, re, :], xh[jj, k, im, :]) for jj in range(NJ)]
                h = [(kh[jj, k, re, :], kh[jj, k, im, :]) for jj in range(NJ)]
                fold = _cadd_i if i < 2 else _csub_i
                h = ([(h[0][0] + vec_s[c, KS:KS + 1, :], h[0][1])]
                     + [fold(h[m], h[m - 1]) for m in range(1, NJ)])
                for jj in range(NJ):
                    acc = _cmul(h[jj], x[0])
                    for j in range(1, jj + 1):
                        acc = _cadd(acc, _cmul(h[jj - j], x[j]))
                    yh[jj, k, re, :] = acc[0]
                    yh[jj, k, im, :] = acc[1]
            return run
        return [item(i, k) for i in range(C // 8 // NJ) for k in range(R)]

    def inv_items(c, slot, jj):
        def run():
            spec = _dft4([yh_s[slot][jj, k] for k in range(R)], +1)
            dst = y_s.at[c, pl.ds(_aligned(jj * R * C, R * C), R * C + SPARE), :]
            for j in range(R):
                g = jnp.concatenate([_ld16(g_ref, 2 * j * C, C),
                                     _ld16(g_ref, (2 * j + 1) * C, C)], axis=1)
                dst[pl.ds(j, C, stride=R), :] = jnp.dot(g, spec[j].astype(BF16),
                                                        preferred_element_type=F32)
        return [run]

    def gate_items(t0, rows):
        src = x_v.at[:, pl.ds(_aligned(t0 // 2, 8), rows // 2), :]
        dst = gate_s.at[pl.ds(_aligned(t0, 8), rows), :]

        def item(r0):
            def run():
                z = _ld16(src.at[0], r0, AR).astype(F32) * vec_s[0, KS + 1:KS + 2, :]
                for c in range(1, NT):
                    z = z + _ld16(src.at[c], r0, AR).astype(F32) * vec_s[c, KS + 1:KS + 2, :]
                z = jnp.sum(z, axis=-1, keepdims=True)
                dst[pl.ds(r0, AR), :] = jnp.broadcast_to(1.0 / (1.0 + jnp.exp(-z)), (AR, LANES))
            return run
        return [item(r0) for r0 in range(0, rows, AR)]

    def mix_items(s):
        words = pl.ds(_aligned(s * (TB // 2), TB // 2), TB // 2)
        rows = pl.ds(_aligned(s * TB, TB), TB)
        x, out = x_v.at[:, words, :], out_v.at[:, words, :]
        att, y, gates = b_s.at[:, rows, :], y_s.at[:, rows, :], gate_s.at[rows, :]

        def item(r0):
            def run():
                gate = gates[pl.ds(r0, MR), :]
                for c in range(NT):
                    b = att[c, pl.ds(r0, MR), :]
                    a = _ld16(x.at[c], r0, MR).astype(F32) * y[c, pl.ds(r0, MR), :]
                    _st16(out.at[c], r0, gate * (a - b) + b)
            return run
        return [item(r0) for r0 in range(0, TB, MR)]

    def emit(*lists):
        for run in _interleave(*lists):
            run()

    start(w_copies(0) + x_copies(0))
    small = jnp.concatenate([sk_ref[...].astype(F32), d_ref[...].astype(F32).reshape(1, D),
                             gw_ref[...].astype(F32).reshape(1, D), jnp.zeros((2, D), F32)], axis=0)
    for c in range(NT):
        vec_s[c] = small[:, c * LANES:(c + 1) * LANES]
        k_v[c, pl.ds(0, 8), :] = jnp.zeros((8, LANES), U32)

    def first_weights(c):
        wait(w_copies(0, [c]))
        if c == 0:
            start(w_copies(1) + x_copies(1))

    prep_wqkv(0, first_weights)
    wait(x_copies(0))
    start(w_copies(2))
    emit(dense_items(0, 0, x_v, qkv_block(0, 0)))
    wait(x_copies(1))
    start(tile_copies(0))

    @pl.loop(0, 2)
    def _(p):
        wait(w_copies(p + 1))
        emit(dense_items(p, 1 - p, x_v, qkv_block(p, 1 - p)), [lambda: prep_wqkv(p + 1)])

    start(x_copies(2) + x_copies(3) + w_copies(3))
    emit(dense_items(2, 0, x_v, qkv_block(2, 0)))
    for p in (1, 2):
        for c in range(NT):
            qkv_s[p, c, pl.ds(0, HALO), :] = jnp.broadcast_to(
                qkv_s[p, c, pl.ds(HALO, 1), :], (HALO, LANES))

    first_rows, tick_rows = TB // NJ, 80
    assert TB + (NT - 1) * NJ * tick_rows == O_SPLIT * TB
    done = 4

    def stage_copy(i):
        return pltpu.make_async_copy(stage_s.at[i % STAGES], qkv_block((i + done) % 3, (i + done) // 3),
                                     stage_sem.at[i % STAGES])

    def tick(c, u, slot, mac, inv, first=False):
        i = c * NJ + u
        p, s = (i + done) % 3, (i + done) // 3

        @pl.when(i >= STAGES)
        def _():
            stage_copy(i - STAGES).wait()

        @pl.when(p == 0)
        def _():
            wait(x_copies(s))

            @pl.when(s + 2 < NB)
            def _():
                start(x_copies(s + 2))

        pl.when(u == 0)(lambda: wait(tile_copies(c)))
        pl.when(jnp.logical_and(u == 0, c + 1 < NT))(lambda: start(tile_copies(c + 1)))

        lists = [dense_items(p, s, x_v, stage_s.at[i % STAGES]), fwd_items(c, slot, u)]
        if inv:
            lists.append(inv_items(c - 2, slot, u))
        t0, rows = ((i * first_rows, first_rows) if first
                    else (TB + (i - NJ) * tick_rows, tick_rows))
        lists.append(attn_items(t0, rows, o0_s, 0, first))
        lists.append(gate_items(t0, rows))
        if mac:
            lists.append(mac_items(c - 1, 1 - slot, u))
        emit(*lists)
        stage_copy(i).start()

    def ticks(c, slot, **stages):
        pl.loop(0, NJ)(lambda u: tick(c, u, slot, **stages))

    ticks(0, 0, mac=False, inv=False, first=True)
    wait(w_copies(3))
    prep_wo()
    ticks(1, 1, mac=True, inv=False)

    @pl.loop(2, NT)
    def _(c):
        for slot in range(2):
            pl.when(c % 2 == slot)(lambda: ticks(c, slot, mac=True, inv=True))

    for i in range(NT * NJ - STAGES, NT * NJ):
        stage_copy(i).wait()

    def out_items(s, o_ref, o_block0):
        return dense_items(3, s - o_block0, o_ref, b_s.at[:, pl.ds(_aligned(s * TB, TB), TB), :])

    @pl.loop(0, NJ)
    def _(u):
        t0 = O_SPLIT * TB + u * tick_rows
        emit(out_items(u, o0_s, 0), inv_items(NT - 2, NT % 2, u),
             attn_items(t0, tick_rows, o1_s, O_SPLIT * TB), gate_items(t0, tick_rows),
             mac_items(NT - 1, (NT - 1) % 2, u))

    done_rows = O_SPLIT * TB + NJ * tick_rows
    for s, rows, chunks, mixed in ((4, 64, (0, 1), ()), (5, 64, (2,), (0, 1, 2)),
                                   (6, 64, (3,), (3, 4)), (7, 0, (), (5, 6))):
        emit(out_items(s, o0_s, 0) if s < O_SPLIT else out_items(s, o1_s, O_SPLIT),
             [it for jj in chunks for it in inv_items(NT - 1, (NT - 1) % 2, jj)],
             attn_items(done_rows, rows, o1_s, O_SPLIT * TB) if rows else [],
             gate_items(done_rows, rows) if rows else [],
             [it for m in mixed for it in mix_items(m)])
        done_rows += rows
        for m in mixed:
            start(out_copies(m))
    assert done_rows == S
    emit(mix_items(NB - 1))
    start(out_copies(NB - 1))
    for s in range(NB):
        wait(out_copies(s))


@jax.jit
def pallas_gated_mix__ssm_conv_h3__sliding_local_dilated__prompt_kernel(
    A_q: jax.Array,
    A_k: jax.Array,
    A_v: jax.Array,
    A_shift_k: jax.Array,
    A_ssm_k: jax.Array,
    A_ssm_D: jax.Array,
    B_x: jax.Array,
    B_wqkv: jax.Array,
    B_wo: jax.Array,
    gate_w: jax.Array,
):
    del B_x
    fwd, inv = _dft_matrices()
    hbm = pl.BlockSpec(memory_space=pl.ANY)
    vmem = pl.BlockSpec(memory_space=pltpu.VMEM)
    out = pl.pallas_call(
        _kernel,
        out_shape=jax.ShapeDtypeStruct((S, D), A_q.dtype),
        in_specs=[hbm, hbm, hbm, vmem, hbm, vmem, hbm, hbm, vmem, vmem, vmem],
        out_specs=hbm,
        scratch_shapes=[
            pltpu.VMEM((NT, S // 2, LANES), U32),
            pltpu.VMEM((NT, 8 + S // 2 + SPARE, LANES), U32),
            pltpu.VMEM((NT, S // 2 + SPARE, LANES), U32),
            pltpu.VMEM((NT, NJ, LANES // 2, R * C), U32),
            pltpu.VMEM((4, NT, D // 2, LANES), U32),
            pltpu.VMEM((NT, S // 2, LANES), U32),
            pltpu.VMEM((NT, D + SPARE, LANES), F32),
            pltpu.VMEM((4, NT, D // 2, LANES), U32),
            pltpu.VMEM((3, NT, HALO + S, LANES), F32),
            pltpu.VMEM((STAGES, NT, TB, LANES), F32),
            pltpu.VMEM((NT, O_SPLIT * TB // 2, LANES), U32),
            pltpu.VMEM((NT, (NB - O_SPLIT) * TB // 2, LANES), U32),
            pltpu.VMEM((NT, S, LANES), F32),
            pltpu.VMEM((R * C // 2 + SPARE, LANES), U32),
            *[pltpu.VMEM((NJ, R, 2 * C, LANES), F32)] * 6,
            pltpu.VMEM((NT, S + SPARE, LANES), F32),
            pltpu.VMEM((S, LANES), F32),
            pltpu.VMEM((NT, 8, LANES), F32),
            pltpu.SemaphoreType.DMA((NB, NT)),
            pltpu.SemaphoreType.DMA((4, NT)),
            pltpu.SemaphoreType.DMA((NT, NJ + 2)),
            pltpu.SemaphoreType.DMA((STAGES,)),
            pltpu.SemaphoreType.DMA((NB, NT)),
        ],
        compiler_params=pltpu.CompilerParams(
            flags={'XLA_TPU_EVENLY_DISTRIBUTE_CRITICAL_NODES': True},
            vmem_limit_bytes=110 * 1024 * 1024),
    )(
        A_q.reshape(S, D), A_k.reshape(S, D), A_v.reshape(S, D),
        A_shift_k.T, A_ssm_k, A_ssm_D, B_wqkv, B_wo,
        gate_w, fwd, inv,
    )
    return out.reshape(A_q.shape)
```
